```python
import os as _os
_os.environ.setdefault("JAX_PLATFORMS", "cpu")
import jax
import jax.numpy as jnp

def _softmax(x, axis=-1):
    return jax.nn.softmax(x, axis=axis)
def _gelu(x):
    return jax.nn.gelu(x, approximate=True)
def _silu(x):
    return jax.nn.silu(x)
def _sigmoid(x):
    return jax.nn.sigmoid(x)
def _layernorm(x, axis=-1, eps=1e-5):
    m = jnp.mean(x, axis=axis, keepdims=True)
    v = jnp.var(x, axis=axis, keepdims=True)
    return (x - m) / jnp.sqrt(v + eps)
def _scatter_add(tgt, idx, src, axis=0):
    return tgt.at[idx].add(src)
def _segment_sum(src, seg, n):
    return jax.ops.segment_sum(src, seg, n)
class _Rng:
    def __init__(self, key):
        self._k = key
    def _next(self):
        self._k, sub = jax.random.split(self._k)
        return sub
    def normal(self, shape):
        return jax.random.normal(self._next(), shape, dtype=jnp.bfloat16)
    def randint(self, lo, hi, shape):
        return jax.random.randint(self._next(), shape, lo, hi, dtype=jnp.int32)
    def uniform(self, shape, lo=0.0, hi=1.0):
        return jax.random.uniform(self._next(), shape, jnp.bfloat16, lo, hi)
    def permutation(self, n):
        return jax.random.permutation(self._next(), n)


kernel_name = 'sequential_preLN__softmax_full_mha__geglu_ffn__prompt'

def setup_inputs():
    _rng = _Rng(jax.random.key(int.from_bytes(__import__("os").urandom(4), "little")))
    _w = (lambda a: (lambda t: t.astype(jnp.bfloat16) if jnp.issubdtype(t.dtype, jnp.floating) else t)(jnp.asarray(a)))
    def _A_setup():
        B, S, D = 1, 2048, 512
        return {
            "x": _w((lambda *s: _rng.normal(s) * 0.05)(B, S, D)),
            "wqkv": _w((lambda *s: _rng.normal(s) * 0.05)(D, 3 * D)),
            "wo": _w((lambda *s: _rng.normal(s) * 0.05)(D, D)),
        }
    _A_in = _A_setup()

    def _B_setup():
        B, S, D, F = 1, 2048, 512, 1376
        return {
            "x": _w((lambda *s: _rng.normal(s) * 0.05)(B, S, D)),
            "w_gate": _w((lambda *s: _rng.normal(s) * 0.05)(D, F)),
            "w_up": _w((lambda *s: _rng.normal(s) * 0.05)(D, F)),
            "w_down": _w((lambda *s: _rng.normal(s) * 0.05)(F, D)),
        }
    _B_in = _B_setup()

    return {
        "A_x": _A_in["x"],
        "A_wqkv": _A_in["wqkv"],
        "A_wo": _A_in["wo"],
        "B_x": _B_in["x"],
        "B_w_gate": _B_in["w_gate"],
        "B_w_up": _B_in["w_up"],
        "B_w_down": _B_in["w_down"],
    }

def reference(A_x, A_wqkv, A_wo, B_x, B_w_gate, B_w_up, B_w_down):
    def _A_ref(x, wqkv, wo):
        B, S, D = x.shape
        H = 32; Dh = D // H
        qkv = (lambda x, *d: x.transpose(*d))((x @ wqkv).reshape(B, S, 3, H, Dh), 2, 0, 3, 1, 4)
        q, k, v = qkv[0], qkv[1], qkv[2]
        scale = Dh ** -0.5
        scores = jnp.einsum("bhqd,bhkd->bhqk", q, k) * scale
        p = _softmax(scores, axis=-1)
        o = jnp.einsum("bhqk,bhkd->bhqd", p, v)
        return (lambda x, *d: x.transpose(*d))(o, 0, 2, 1, 3).reshape(B, S, D) @ wo

    def _B_ref(x, w_gate, w_up, w_down):
        return (_gelu(x @ w_gate) * (x @ w_up)) @ w_down

    x = A_x
    h = x + _A_ref(_layernorm(x, axis=-1), A_wqkv, A_wo)
    h2 = h + _B_ref(_layernorm(h, axis=-1), B_w_gate, B_w_up, B_w_down)
    return h2
```

```python
import functools
import math

import jax
import jax.numpy as jnp
import jax.experimental.pallas as pl
import jax.experimental.pallas.tpu as pltpu

H = 32
DH = 16
HPG = 128 // DH
EPS = 1e-5
TQ = 512
TK = 128
TP = 512

F32 = jnp.float32
BF16 = jnp.bfloat16


def _layernorm(x):
    m = jnp.mean(x, axis=-1, keepdims=True)
    d = x - m
    v = jnp.mean(d * d, axis=-1, keepdims=True)
    return d * jax.lax.rsqrt(v + EPS)


def _gelu_tanh(x):
    c = math.sqrt(2.0 / math.pi)
    return 0.5 * x * (1.0 + jnp.tanh(c * (x + 0.044715 * (x * x * x))))


def _dot(a, b):
    return jnp.dot(a, b, preferred_element_type=F32)


def _kernel(x_ref, wqkv_ref, wo_hbm, wg_hbm, wu_hbm, wd_hbm, o_ref,
            k_s, qt_s, vt_s, s0, s1, ot_s, wo_s, wg_s, wu_s, wd_s, sems,
            *, S, D):
    step = pl.program_id(0)
    G = D // 128
    n_chunks = S // TK
    q_scale = (DH ** -0.5) * math.log2(math.e)

    weight_copies = [
        pltpu.make_async_copy(src, dst, sems.at[i])
        for i, (src, dst) in enumerate(
            [(wo_hbm, wo_s), (wg_hbm, wg_s), (wu_hbm, wu_s), (wd_hbm, wd_s)])
    ]

    @pl.when(step == 0)
    def _():
        for cp in weight_copies:
            cp.start()
        for c in range(S // TP):
            rows = pl.ds(c * TP, TP)
            xn = _layernorm(x_ref[rows, :].astype(F32)).astype(BF16)
            k = _dot(xn, wqkv_ref[:, D:2 * D]).astype(BF16)
            for g in range(G):
                k_s[g, rows, :] = k[:, g * 128:(g + 1) * 128]
            qt = (_dot(xn, wqkv_ref[:, 0:D]) * q_scale).T.astype(BF16)
            for t in range(TP // TQ):
                qt_s[c * (TP // TQ) + t] = qt[:, t * TQ:(t + 1) * TQ].reshape(G, 128, TQ)
            vt = _dot(xn, wqkv_ref[:, 2 * D:3 * D]).T.astype(BF16)
            vt_s[:, :, rows] = vt.reshape(H, DH, TP)

    row_head = jax.lax.broadcasted_iota(jnp.int32, (128, TQ), 0) // DH

    def masked_q(h):
        qt = qt_s[step, h // HPG]
        return jnp.where(row_head == h % HPG, qt, jnp.zeros_like(qt))

    def qk_chunk(h, qm, c, s_ref, m8):
        rows = pl.ds(c * TK, TK)
        s = _dot(k_s[h // HPG, rows, :], qm)
        s_ref[rows, :] = s
        mc = jnp.max(s.reshape(TK // 8, 8, TQ), axis=0)
        return mc if m8 is None else jnp.maximum(m8, mc)

    def pv_chunk(h, c, s_ref, m, acc, l8):
        rows = pl.ds(c * TK, TK)
        p = jnp.exp2(s_ref[rows, :] - m)
        lc = jnp.sum(p.reshape(TK // 8, 8, TQ), axis=0)
        o = _dot(vt_s[h, :, rows], p.astype(BF16))
        if acc is None:
            return o, lc
        return acc + o, l8 + lc

    def stage(h_qk, s_qk, h_pv, s_pv, m):
        m8 = acc = l8 = None
        qm = masked_q(h_qk) if h_qk is not None else None
        for c in range(n_chunks):
            if h_qk is not None:
                m8 = qk_chunk(h_qk, qm, c, s_qk, m8)
            if h_pv is not None:
                acc, l8 = pv_chunk(h_pv, c, s_pv, m, acc, l8)
        if h_pv is not None:
            l = jnp.sum(l8, axis=0, keepdims=True)
            ot_s[h_pv] = acc * (1.0 / l)
        if h_qk is not None:
            return jnp.max(m8, axis=0, keepdims=True)
        return None

    m_first = stage(0, s0, None, None, None)

    def pair(j, m0):
        h = 2 * j
        m1 = stage(h + 1, s1, h, s0, m0)
        return stage(h + 2, s0, h + 1, s1, m1)

    m0 = jax.lax.fori_loop(0, H // 2 - 1, pair, m_first)
    m1 = stage(H - 1, s1, H - 2, s0, m0)
    stage(None, None, H - 1, s1, m1)

    @pl.when(step == 0)
    def _():
        for cp in weight_copies:
            cp.wait()

    o = ot_s[...].reshape(D, TQ).T.astype(BF16)
    rows = pl.ds(pl.multiple_of(step * TQ, TQ), TQ)
    h1 = x_ref[rows, :].astype(F32) + _dot(o, wo_s[...])
    hn = _layernorm(h1).astype(BF16)
    act = (_gelu_tanh(_dot(hn, wg_s[...])) * _dot(hn, wu_s[...])).astype(BF16)
    o_ref[...] = (h1 + _dot(act, wd_s[...])).astype(o_ref.dtype)


@jax.jit
def pallas_sequential_preLN__softmax_full_mha__geglu_ffn__prompt_kernel(
    A_x: jax.Array,
    A_wqkv: jax.Array,
    A_wo: jax.Array,
    B_x: jax.Array,
    B_w_gate: jax.Array,
    B_w_up: jax.Array,
    B_w_down: jax.Array,
):
    B, S, D = A_x.shape
    F = B_w_gate.shape[1]
    assert B == 1 and D == H * DH and S % TP == 0 and TP % TQ == 0
    x = A_x.reshape(S, D)
    G = D // 128

    out = pl.pallas_call(
        functools.partial(_kernel, S=S, D=D),
        grid=(S // TQ,),
        in_specs=[
            pl.BlockSpec((S, D), lambda i: (0, 0)),
            pl.BlockSpec((D, 3 * D), lambda i: (0, 0)),
            pl.BlockSpec(memory_space=pl.ANY),
            pl.BlockSpec(memory_space=pl.ANY),
            pl.BlockSpec(memory_space=pl.ANY),
            pl.BlockSpec(memory_space=pl.ANY),
        ],
        out_specs=pl.BlockSpec((TQ, D), lambda i: (i, 0)),
        out_shape=jax.ShapeDtypeStruct((S, D), A_x.dtype),
        scratch_shapes=[
            pltpu.VMEM((G, S, 128), BF16),
            pltpu.VMEM((S // TQ, G, 128, TQ), BF16),
            pltpu.VMEM((H, DH, S), BF16),
            pltpu.VMEM((S, TQ), F32),
            pltpu.VMEM((S, TQ), F32),
            pltpu.VMEM((H, DH, TQ), F32),
            pltpu.VMEM((D, D), BF16),
            pltpu.VMEM((D, F), BF16),
            pltpu.VMEM((D, F), BF16),
            pltpu.VMEM((F, D), BF16),
            pltpu.SemaphoreType.DMA((4,)),
        ],
        compiler_params=pltpu.CompilerParams(
            dimension_semantics=("arbitrary",),
            vmem_limit_bytes=100 * 1024 * 1024,
        ),
    )(x, A_wqkv, A_wo, B_w_gate, B_w_up, B_w_down)
    return out.reshape(B, S, D)
```

```python
import functools
import math

import jax
import jax.numpy as jnp
import jax.experimental.pallas as pl
import jax.experimental.pallas.tpu as pltpu

H = 32
DH = 16
HPG = 128 // DH
EPS = 1e-5
TQ = 512
TK = 128
TP = 512
TF = 512
LEAD = 3
FILL0 = 8
SCORE_LIMIT = 64.0
VALUE_LIMIT = 2.0 ** 30

F32 = jnp.float32
BF16 = jnp.bfloat16
U32 = jnp.uint32


def _layernorm(x):
    m = jnp.mean(x, axis=-1, keepdims=True)
    d = x - m
    v = jnp.mean(d * d, axis=-1, keepdims=True)
    return d * jax.lax.rsqrt(v + EPS)


def _gelu_tanh(x):
    c = math.sqrt(2.0 / math.pi)
    return 0.5 * x * (1.0 + jnp.tanh(c * (x + 0.044715 * (x * x * x))))


def _dot(a, b):
    return jnp.dot(a, b, preferred_element_type=F32)


def _dot_nt(a, b):
    return jax.lax.dot_general(a, b, (((1,), (1,)), ((), ())),
                               preferred_element_type=F32)


def _pack(x):
    return pltpu.bitcast(x, U32)


def _unpack(x):
    return pltpu.bitcast(x, BF16)


def _abs_slab_max(x):
    a = jnp.abs(x)
    m = a[:, 0:128]
    for g in range(1, x.shape[1] // 128):
        m = jnp.maximum(m, a[:, g * 128:(g + 1) * 128])
    return m


def _rows_max8(x):
    return jnp.max(x.reshape(x.shape[0] // 8, 8, x.shape[1]), axis=0)


def _head_norm_bound(x):
    m = _abs_slab_max(x)
    m = m * m
    sh = DH // 2
    while sh:
        m = m + pltpu.roll(m, sh, 1)
        sh //= 2
    return _rows_max8(m)


def _kernel(x_hbm, wqkv_hbm, wo_hbm, wg_hbm, wu_hbm, wd_hbm, o_ref,
            x_s, wqkv_s, k_s, qt_s, vt_s, qf_s, kh0, kh1, kb0, kb1, sc_s, ot_s,
            wo_s, wg_s, wu_s, wd_s, sems, *, S, D):
    step = pl.program_id(0)
    G = D // 128
    NC = S // TK
    NT = S // TQ
    NG = TK // 16
    NJ = TQ // 128
    NP = S // TP
    q_scale = (DH ** -0.5) * math.log2(math.e)

    x_copies = [
        pltpu.make_async_copy(x_hbm.at[pl.ds(i * TP, TP)], x_s.at[pl.ds(i * TP, TP)],
                              sems.at[i])
        for i in range(NP)]
    w_copies = [
        pltpu.make_async_copy(wqkv_hbm.at[:, pl.ds(i * D, D)], wqkv_s.at[i],
                              sems.at[NP + i])
        for i in range(3)]
    late_copies = [
        pltpu.make_async_copy(src, dst, sems.at[NP + 3 + i])
        for i, (src, dst) in enumerate(
            [(wo_hbm, wo_s), (wg_hbm, wg_s), (wu_hbm, wu_s), (wd_hbm, wd_s)])
    ]

    def prep_keys(slab, shift, c, kh, kb):
        if shift is not None:
            slab = pltpu.roll(slab, shift, 1)
        kh[pl.ds(c * (TK // 2), TK // 2), :] = slab
        ko = _unpack(slab[0:8]).astype(F32)
        for d in range(DH):
            kb[c, d] = jnp.broadcast_to(ko[:, d:d + 1], (16, 128))

    def head_shift(h):
        return (128 - (h % HPG) * DH) % 128

    def project(ci):
        rows = pl.ds(ci * TP, TP)
        x_copies[ci].wait()
        xn = _layernorm(x_s[rows, :].astype(F32)).astype(BF16)
        if ci == 0:
            w_copies[1].wait()
        kf = _dot(xn, wqkv_s[1])
        k = _pack(kf.astype(BF16))
        for g in range(G):
            k_s[g, pl.ds(ci * (TP // 2), TP // 2), :] = k[:, g * 128:(g + 1) * 128]
        n = TP // TK
        for i in range(n):
            prep_keys(k[i * (TK // 2):(i + 1) * (TK // 2), 0:128], None, ci * n + i, kh0, kb0)
        if ci == 0:
            w_copies[0].wait()
        qf = _dot(xn, wqkv_s[0]) * q_scale
        qt = qf.T.astype(BF16)
        qt_s[:, :, rows] = _pack(qt).reshape(H, DH // 2, TP)
        qf_s[:, :, rows] = qt.astype(F32).reshape(H, DH, TP)
        if ci == 0:
            w_copies[2].wait()
        vf = _dot(xn, wqkv_s[2])
        vt_s[:, :, rows] = _pack(vf.T.astype(BF16)).reshape(H, DH // 2, TP)
        return (_head_norm_bound(qf), _head_norm_bound(kf),
                _rows_max8(_abs_slab_max(vf)))

    def store_out(h, qi, acc, l8):
        l = jnp.sum(l8, axis=0, keepdims=True)
        ot_s[qi * TQ // TF, h, :, pl.ds((qi * TQ) % TF, TQ)] = acc * (1.0 / l)

    def vpu_scores(h, qi, c, j, kb, z):
        acc = None
        for d in range(DH):
            qb = jnp.broadcast_to(
                qf_s[h, d:d + 1, pl.ds(qi * TQ + j * 128, 128)], (8, 128))
            t = kb[c + z, d] * jnp.concatenate([qb, qb], axis=0)
            acc = t if acc is None else acc + t
        return acc

    NM = NG - 1

    def head_pair(jj, carry):
        h0 = 2 * jj
        zs = [jnp.minimum(jj, 0) * (j + 1) for j in range(NJ)]
        khs = (kh0, kh1)
        tabs = (kb0, kb1)
        units = [(hh, qi) for hh in range(2) for qi in range(NT)]
        stream = [(c, g) for c in range(NC) for g in reversed(range(1, NG))]
        bounds = [0] + [min((c + 1) * NM + LEAD, NC * NM) for c in range(NC)]
        probs = {}
        lacc = {}
        acc = None
        total = len(units) * NC

        def consume(ui, c, g, j, sg):
            p = jnp.exp2(sg)
            pair = p[0:8] + p[8:16]
            lacc[ui, j] = pair if (ui, j) not in lacc else lacc[ui, j] + pair
            probs[(ui, c, g, j)] = p

        for t in range(total + 1):
            if t < total:
                ui, c = divmod(t, NC)
                hh, qi = units[ui]
                h = h0 + hh
                if c == 0:
                    qh = _unpack(qt_s[h, :, pl.ds(qi * TQ, TQ)])
                part = stream[bounds[c]:bounds[c + 1]]
                kk = jnp.concatenate(
                    [khs[hh][pl.ds(cc * (TK // 2) + 8 * g, 8), :] for cc, g in part], axis=0)
                s = _dot(_unpack(kk)[:, 0:DH], qh)
                at = [(j * len(part)) // NJ for j in range(NJ)]
                for i, (cc, g) in enumerate(part):
                    for j in range(NJ):
                        if at[j] == i:
                            consume(ui, c, 0, j, vpu_scores(h, qi, c, j, tabs[hh], zs[j]))
                    for j in range(NJ):
                        consume(ui, cc, g, j, s[16 * i:16 * (i + 1), 128 * j:128 * (j + 1)])
                i = qi * NC + c - FILL0
                if 0 <= i < 3 * NC and i % 3 == 0:
                    cn = i // 3
                    hn = jnp.minimum(h + 1, H - 1)
                    prep_keys(k_s[hn // HPG, pl.ds(cn * (TK // 2), TK // 2), :],
                              head_shift(hn), cn, khs[1 - hh], tabs[1 - hh])
            u = t - 1
            if u >= 0:
                ui, c = divmod(u, NC)
                hh, qi = units[ui]
                h = h0 + hh
                pt = jnp.concatenate(
                    [jnp.concatenate([probs.pop((ui, c, g, j)) for j in range(NJ)], axis=1)
                     for g in range(NG)], axis=0).astype(BF16)
                o = _dot(_unpack(vt_s[h, :, pl.ds(c * TK, TK)]), pt)
                acc = o if c == 0 else acc + o
                if c == NC - 1:
                    store_out(h, qi, acc,
                              jnp.concatenate([lacc[ui, j] for j in range(NJ)], axis=1))
        return carry

    def safe_head(h, carry):
        kh0[...] = pltpu.roll(k_s[h // HPG], head_shift(h), 1)
        for qi in range(NT):
            qh = _unpack(qt_s[h, :, pl.ds(qi * TQ, TQ)])

            def scores(c, m8):
                r = pl.multiple_of(c * (TK // 2), TK // 2)
                s = _dot(_unpack(kh0[pl.ds(r, TK // 2), :])[:, 0:DH], qh)
                sc_s[c] = s
                return jnp.maximum(m8, _rows_max8(s))

            m8 = jax.lax.fori_loop(0, NC, scores, jnp.full((8, TQ), -jnp.inf, F32))
            m = jnp.max(m8, axis=0, keepdims=True)

            def weigh(c, st):
                acc, l8 = st
                p = jnp.exp2(sc_s[c] - m)
                v = _unpack(vt_s[h, :, pl.ds(pl.multiple_of(c * TK, TK), TK)])
                return (acc + _dot(v, p.astype(BF16)),
                        l8 + jnp.sum(p.reshape(TK // 8, 8, TQ), axis=0))

            acc, l8 = jax.lax.fori_loop(
                0, NC, weigh, (jnp.zeros((DH, TQ), F32), jnp.zeros((8, TQ), F32)))
            store_out(h, qi, acc, l8)
        return carry

    @pl.when(step == 0)
    def _():
        for cp in (x_copies[0], w_copies[1], w_copies[0], w_copies[2]):
            cp.start()
        for cp in x_copies[1:] + late_copies:
            cp.start()
        stats = None
        for ci in range(NP):
            st = project(ci)
            stats = st if stats is None else tuple(
                jnp.maximum(a, b) for a, b in zip(stats, st))
        qn, kn, vmax = (jnp.max(a) for a in stats)
        bounded = jnp.logical_and(qn * kn * 1.05 <= SCORE_LIMIT * SCORE_LIMIT,
                                  vmax <= VALUE_LIMIT)

        @pl.when(bounded)
        def _():
            jax.lax.fori_loop(0, H // 2, head_pair, 0)

        @pl.when(jnp.logical_not(bounded))
        def _():
            jax.lax.fori_loop(0, H, safe_head, 0)

        for cp in late_copies:
            cp.wait()

    o = ot_s[step].reshape(D, TF).T.astype(BF16)
    rows = pl.ds(pl.multiple_of(step * TF, TF), TF)
    h1 = x_s[rows, :].astype(F32) + _dot(o, wo_s[...])
    hn = _layernorm(h1).astype(BF16)
    act = (_gelu_tanh(_dot_nt(hn, wg_s[...])) * _dot_nt(hn, wu_s[...])).astype(BF16)
    o_ref[...] = (h1 + _dot(act, wd_s[...])).astype(o_ref.dtype)


@jax.jit
def pallas_sequential_preLN__softmax_full_mha__geglu_ffn__prompt_kernel(
    A_x: jax.Array,
    A_wqkv: jax.Array,
    A_wo: jax.Array,
    B_x: jax.Array,
    B_w_gate: jax.Array,
    B_w_up: jax.Array,
    B_w_down: jax.Array,
):
    B, S, D = A_x.shape
    F = B_w_gate.shape[1]
    assert B == 1 and D == H * DH and S % TP == 0 and TF % TQ == 0
    x = A_x.reshape(S, D)
    G = D // 128
    NC = S // TK
    hbm = pl.BlockSpec(memory_space=pltpu.MemorySpace.HBM)

    out = pl.pallas_call(
        functools.partial(_kernel, S=S, D=D),
        grid=(S // TF,),
        in_specs=[hbm] * 6,
        out_specs=pl.BlockSpec((TF, D), lambda i: (i, 0)),
        out_shape=jax.ShapeDtypeStruct((S, D), A_x.dtype),
        scratch_shapes=[
            pltpu.VMEM((S, D), BF16),
            pltpu.VMEM((3, D, D), BF16),
            pltpu.VMEM((G, S // 2, 128), U32),
            pltpu.VMEM((H, DH // 2, S), U32),
            pltpu.VMEM((H, DH // 2, S), U32),
            pltpu.VMEM((H, DH, S), F32),
            pltpu.VMEM((S // 2, 128), U32),
            pltpu.VMEM((S // 2, 128), U32),
            pltpu.VMEM((NC, DH, 16, 128), F32),
            pltpu.VMEM((NC, DH, 16, 128), F32),
            pltpu.VMEM((NC, TK, TQ), F32),
            pltpu.VMEM((S // TF, H, DH, TF), F32),
            pltpu.VMEM((D, D), BF16),
            pltpu.VMEM((F, D), BF16),
            pltpu.VMEM((F, D), BF16),
            pltpu.VMEM((F, D), BF16),
            pltpu.SemaphoreType.DMA((S // TP + 7,)),
        ],
        compiler_params=pltpu.CompilerParams(
            dimension_semantics=("arbitrary",),
            vmem_limit_bytes=100 * 1024 * 1024,
        ),
    )(x, A_wqkv, A_wo, B_w_gate.T, B_w_up.T, B_w_down)
    return out.reshape(B, S, D)
```

```python
import functools
import math

import jax
import jax.numpy as jnp
import jax.experimental.pallas as pl
import jax.experimental.pallas.tpu as pltpu

H = 32
DH = 16
HPG = 128 // DH
EPS = 1e-5
TQ = 512
TK = 128
TF = 512
FSPLIT = 2
CHUNKS = (256, 256, 512, 512, 512)
NVP = (3, 3, 2, 2)
LEAD = 3
VOFF = 2
FILL0 = 2
FILL1 = 60
SUM_LIMIT = 2.0 ** 64
VALUE_LIMIT = 2.0 ** 30
FFN_T = 1
PIN = 1
PADR = 1024

F32 = jnp.float32
BF16 = jnp.bfloat16
U32 = jnp.uint32


def _layernorm(x):
    m = jnp.mean(x, axis=-1, keepdims=True)
    d = x - m
    v = jnp.mean(d * d, axis=-1, keepdims=True)
    return d * jax.lax.rsqrt(v + EPS)


def _gelu_tanh(x):
    c = math.sqrt(2.0 / math.pi)
    return 0.5 * x * (1.0 + jnp.tanh(c * (x + 0.044715 * (x * x * x))))


def _dot(a, b):
    return jnp.dot(a, b, preferred_element_type=F32)


def _dot_nt(a, b):
    return jax.lax.dot_general(a, b, (((1,), (1,)), ((), ())),
                               preferred_element_type=F32)


def _abs_slab_max(x):
    a = jnp.abs(x)
    m = a[:, 0:128]
    for g in range(1, x.shape[1] // 128):
        m = jnp.maximum(m, a[:, g * 128:(g + 1) * 128])
    return m


def _rows_max8(x):
    return jnp.max(x.reshape(x.shape[0] // 8, 8, x.shape[1]), axis=0)


def _lane_shift(x, n):
    lane = jax.lax.broadcasted_iota(jnp.int32, x.shape, 1)
    return jnp.take_along_axis(x, (lane + n) & 127, axis=1)


def _kernel(x_hbm, wqkv_hbm, wo_hbm, wg_hbm, wu_hbm, wd_hbm, o_ref,
            x_s, wqkv_s, k_s, kp_s, qt_s, vt_s, kh0, kh1, kb0, kb1, kf_s, sc_s, pend_s, ot_s, l_s, r_s, on_s, ob_s,
            wo_s, wg_s, wu_s, wd_s, sems, osems, *, S, D):
    step = pl.program_id(0)
    G = D // 128
    NC = S // TK
    NT = S // TQ
    NG = TK // 8
    NJ = TQ // 128
    q_scale = (DH ** -0.5) * math.log2(math.e)
    nv = [NVP[c % len(NVP)] for c in range(NC)]
    starts = [sum(CHUNKS[:i]) for i in range(len(CHUNKS))]
    order = [(c, g) for c in range(NC) for g in reversed(range(nv[c], NG))]
    first = [sum(NG - nv[i] for i in range(c)) for c in range(NC + 1)]
    NS = len(order)
    NPAIR = NS // 2

    x_parts = [(starts[i], CHUNKS[i]) for i in range(3)] + [(starts[3], S - starts[3])]
    x_copies = [
        pltpu.make_async_copy(x_hbm.at[pl.ds(r0, n)], x_s.at[pl.ds(r0, n)], sems.at[i])
        for i, (r0, n) in enumerate(x_parts)]
    w_copies = [
        pltpu.make_async_copy(wqkv_hbm.at[:, pl.ds(i * D, D)], wqkv_s.at[i], sems.at[4 + i])
        for i in range(3)]
    late_copies = [
        pltpu.make_async_copy(src, dst, sems.at[7 + i])
        for i, (src, dst) in enumerate(
            [(wo_hbm, wo_s), (wg_hbm, wg_s), (wu_hbm, wu_s), (wd_hbm, wd_s)])
    ]

    def fill_table(rows, lane0, c, ds, kb):
        for d in ds:
            lane = jnp.full(rows.shape, lane0 + d, jnp.int32)
            kb[c, d, 0:rows.shape[0], :] = jnp.take_along_axis(rows, lane, axis=1)

    def norm_rows(ci):
        return _layernorm(x_s[pl.ds(starts[ci], CHUNKS[ci]), :].astype(F32)).astype(BF16)

    def project_k(ci, xn):
        r0, n = starts[ci], CHUNKS[ci]
        c0, c1 = r0 // TK, (r0 + n) // TK
        k = _dot(xn, wqkv_s[1])
        kp = jnp.concatenate(
            [k[(c - c0) * TK + 8 * g:(c - c0) * TK + 8 * g + 8]
             for c, g in order[first[c0]:first[c1]]], axis=0)
        kp = pltpu.bitcast(kp.astype(BF16), U32)
        prows = pl.ds(first[c0] * 4, (first[c1] - first[c0]) * 4)
        for g in range(G):
            k_s[g, pl.ds(r0, n), :] = k[:, g * 128:(g + 1) * 128]
            kp_s[g, prows, :] = kp[:, g * 128:(g + 1) * 128]
        kh0[prows, :] = kp[:, 0:128]
        for c in range(c0, c1):
            r = (c - c0) * TK
            fill_table(k[r:r + 8 * nv[c], 0:128], 0, c, range(DH), kb0)

    def project_q(ci, xn):
        r0, n = starts[ci], CHUNKS[ci]
        q = _dot(xn, wqkv_s[0]) * q_scale
        qt_s[:, :, pl.ds(r0, n)] = q.T.reshape(H, DH, n)

    def project_v(ci, xn):
        r0, n = starts[ci], CHUNKS[ci]
        v = _dot(xn, wqkv_s[2])
        vt_s[:, :, pl.ds(r0, n)] = v.T.reshape(H, DH, n)

    def store_out(h, qi, acc, l8):
        cols = pl.ds((qi * TQ) % TF, TQ)
        ot_s[qi * TQ // TF, h, :, cols] = acc
        for j in range(NJ):
            l_s[qi * NJ + j, pl.ds(pl.multiple_of(h * 8, 8), 8), :] = (
                l8[:, 128 * j:128 * (j + 1)])

    def stage_attn(blk):
        for j in range(TF // 128):
            t = blk * (TF // 128) + j
            l = l_s[t, pl.ds(0, H, stride=8), :]
            for i in range(1, 8):
                l = l + l_s[t, pl.ds(i, H, stride=8), :]
            r_s[:, 128 * j:128 * (j + 1)] = 1.0 / l
        heads = []
        for h in range(H):
            r = jnp.concatenate(
                [jnp.broadcast_to(r_s[h:h + 1, 128 * j:128 * (j + 1)], (8, 128))
                 for j in range(TF // 128)], axis=1)
            heads.append(ot_s[blk, h] * jnp.concatenate([r, r], axis=0))
        on_s[...] = pltpu.bitcast(jnp.concatenate(heads, axis=0).T.astype(BF16), U32)

    def vpu_scores(h, qi, c, j, kb, z):
        accs = [None] * nv[c]
        for d in range(DH):
            qb = jnp.broadcast_to(
                qt_s[h, d:d + 1, pl.ds(qi * TQ + j * 128, 128)], (8, 128))
            for g in range(nv[c]):
                t = kb[c + z, d, 8 * g:8 * (g + 1), :] * qb
                accs[g] = t if accs[g] is None else accs[g] + t
        return accs

    def prep_piece(h, pc, kh, kb):
        g, lane0 = h // HPG, (h % HPG) * DH
        lo, hi = (pc * NPAIR) // (4 * NC), ((pc + 1) * NPAIR) // (4 * NC)
        rows = pl.ds(8 * lo, 8 * (hi - lo))
        kh[rows, :] = _lane_shift(kp_s[g, rows, :], lane0)
        c, part = divmod(pc, 4)
        fill_table(k_s[g, pl.ds(c * TK, 8 * nv[c]), :], lane0, c,
                   range(part * (DH // 4), (part + 1) * (DH // 4)), kb)

    def finish_pending(h, zs, state):
        lmin, lmax, acc, l8 = state
        n = nv[NC - 1]
        cols, sums = [], []
        for j in range(NJ):
            ps = [jnp.exp2(sv) for sv in vpu_scores(h, NT - 1, NC - 1, j, kb1, zs[j])]
            lj = l8[:, 128 * j:128 * (j + 1)]
            for p in ps:
                lj = lj + p
            lmin = jnp.minimum(lmin, lj)
            lmax = jnp.maximum(lmax, lj)
            cols.append(jnp.concatenate(ps, axis=0))
            sums.append(lj)
        pt = jnp.concatenate(
            [jnp.concatenate(cols, axis=1), pend_s[pl.ds(8 * n, TK - 8 * n), :]], axis=0)
        o = _dot(vt_s[h, :, pl.ds((NC - 1) * TK, TK)], pt)
        store_out(h, NT - 1, acc + o, jnp.concatenate(sums, axis=1))
        return lmin, lmax

    def head_pair(jj, carry):
        h0 = 2 * jj
        zs = [jnp.minimum(jj, 0) * (j + 1) for j in range(NJ)]
        zero = zs[0].astype(F32)
        khs = (kh0, kh1)
        tabs = (kb0, kb1)
        units = [(hh, qi) for hh in range(2) for qi in range(NT)]
        total = len(units) * NC
        slen = len(units) * NS
        ends = [(t // NC) * NS + first[t % NC + 1] for t in range(total)]
        cuts = [min(e + LEAD + (e + LEAD) % 2, slen) for e in ends]
        pieces = {}
        work = sum(nv) * NJ * len(units)
        done = 0
        for t in range(total - 1):
            for j in range(NJ):
                pos = (done * slen) // work + VOFF
                pos = max(0, min(pos, cuts[t] - 1))
                pieces.setdefault(pos, []).append((t, j))
                done += nv[t % NC]
        probs = {}
        lacc = {}
        qhs = {}
        acc = None

        def consume(t, g, j, sg):
            p = jnp.exp2(sg)
            key = (t // NC, j)
            lacc[key] = p if key not in lacc else lacc[key] + p
            probs[(t, g, j)] = p

        def score_rows(lo, hi):
            ui = lo // NS
            hh, qi = units[ui]
            if ui not in qhs:
                qhs[ui] = qt_s[h0 + hh, :, pl.ds(qi * TQ, TQ)].astype(BF16)
            kk = pltpu.bitcast(khs[hh][pl.ds(4 * (lo - ui * NS), 4 * (hi - lo)), :], BF16)
            s = _dot(kk[:, 0:DH], qhs[ui])
            for i in range(lo, hi):
                for tv, j in pieces.get(i, ()):
                    hv, qv = units[tv // NC]
                    sv = vpu_scores(h0 + hv, qv, tv % NC, j, tabs[hv], zs[j])
                    for gv in reversed(range(len(sv))):
                        consume(tv, gv, j, sv[gv])
                c, g = order[i - ui * NS]
                r = 8 * (i - lo)
                for j in range(NJ):
                    consume(ui * NC + c, g, j, s[r:r + 8, 128 * j:128 * (j + 1)])

        lo = 0
        for t in range(total + 1):
            if t < total:
                hi = cuts[t]
                cut = ends[t] if (t % NC == NC - 1 and hi > ends[t]) else hi
                if cut > lo:
                    score_rows(lo, cut)
                if hi > cut:
                    score_rows(cut, hi)
                lo = hi
                hh, qi = units[t // NC]
                i = qi * NC + t % NC
                hn = jnp.minimum(h0 + hh + 1, H - 1)
                for pc in range(4 * NC):
                    if FILL0 + (pc * (FILL1 - FILL0)) // (4 * NC) == i:
                        prep_piece(hn, pc, khs[1 - hh], tabs[1 - hh])
            u = t - 1
            if u < 0:
                lmin, lmax = finish_pending(jnp.maximum(h0 - 1, 0), zs, carry)
            else:
                ui, c = divmod(u, NC)
                hh, qi = units[ui]
                h = h0 + hh
                g0 = nv[c] if u == total - 1 else 0
                pt = jnp.concatenate(
                    [jnp.concatenate([probs.pop((u, g, j)) for j in range(NJ)], axis=1)
                     for g in range(g0, NG)], axis=0)
                l8 = None
                if c == NC - 1:
                    l8 = jnp.concatenate([lacc[ui, j] for j in range(NJ)], axis=1)
                if u == total - 1:
                    pend_s[pl.ds(8 * g0, TK - 8 * g0), :] = pt
                    continue
                o = _dot(vt_s[h, :, pl.ds(c * TK, TK)], pt)
                acc = (zero if c == 0 else acc) + o
                if c == NC - 1:
                    for j in range(NJ):
                        lmin = jnp.minimum(lmin, lacc[ui, j])
                        lmax = jnp.maximum(lmax, lacc[ui, j])
                    store_out(h, qi, acc, l8)
        return lmin, lmax, acc, l8

    def safe_head(h, carry):
        def shift_keys(c, carry):
            rows = pl.ds(pl.multiple_of(c * TK, TK), TK)
            kf_s[rows, :] = _lane_shift(k_s[h // HPG, rows, :], (h % HPG) * DH)
            return carry

        jax.lax.fori_loop(0, NC, shift_keys, 0)
        for qi in range(NT):
            qh = qt_s[h, :, pl.ds(qi * TQ, TQ)]

            def scores(c, m8):
                s = _dot(kf_s[pl.ds(pl.multiple_of(c * TK, TK), TK), :][:, 0:DH], qh)
                sc_s[c] = s
                return jnp.maximum(m8, _rows_max8(s))

            m8 = jax.lax.fori_loop(0, NC, scores, jnp.full((8, TQ), -jnp.inf, F32))
            m = jnp.max(m8, axis=0, keepdims=True)

            def weigh(c, st):
                acc, l8 = st
                p = jnp.exp2(sc_s[c] - m)
                v = vt_s[h, :, pl.ds(pl.multiple_of(c * TK, TK), TK)]
                return (acc + _dot(v, p),
                        l8 + jnp.sum(p.reshape(TK // 8, 8, TQ), axis=0))

            acc, l8 = jax.lax.fori_loop(
                0, NC, weigh, (jnp.zeros((DH, TQ), F32), jnp.zeros((8, TQ), F32)))
            store_out(h, qi, acc, l8)
        return carry

    @pl.when(step == 0)
    def _():
        for cp in (x_copies[0], w_copies[1], x_copies[1], w_copies[0], w_copies[2],
                   x_copies[2], x_copies[3]):
            cp.start()
        pend_s[...] = jnp.zeros(pend_s.shape, F32)
        kb1[NC - 1] = jnp.zeros(kb1.shape[1:], F32)
        x_copies[0].wait()
        xn0 = norm_rows(0)
        w_copies[1].wait()
        project_k(0, xn0)
        x_copies[1].wait()
        w_copies[0].wait()
        project_q(0, xn0)
        xn1 = norm_rows(1)
        project_q(1, xn1)
        project_k(1, xn1)
        w_copies[2].wait()
        x_copies[2].wait()
        project_v(0, xn0)
        project_v(1, xn1)
        wv8 = _rows_max8(_abs_slab_max(wqkv_s[2].astype(F32)))
        xn = norm_rows(2)
        project_v(2, xn)
        project_k(2, xn)
        x_copies[3].wait()
        for cp in late_copies:
            cp.start()
        project_q(2, xn)
        for ci in range(3, len(CHUNKS)):
            xn = norm_rows(ci)
            project_v(ci, xn)
            project_q(ci, xn)
            project_k(ci, xn)

        ones = jnp.ones((8, 128), F32)
        state = jax.lax.fori_loop(
            0, H // 2, head_pair,
            (ones, ones, jnp.zeros((DH, TQ), F32), jnp.zeros((8, TQ), F32)))
        lmin, lmax = finish_pending(H - 1, [0] * NJ, state)
        stage_attn(0)
        worst = jnp.maximum(jnp.maximum(lmax, 1.0 / lmin) * (1.0 / SUM_LIMIT),
                            wv8 * (D / VALUE_LIMIT))
        wv_max = jnp.max(worst)
        bounded = wv_max <= 1.0

        @pl.when(jnp.logical_not(bounded))
        def _():
            jax.lax.fori_loop(0, H, safe_head, 0)
            stage_attn(0)

        for cp in late_copies:
            cp.wait()

    R = TF // FSPLIT
    h1s, acts = [], []
    for b in range(FSPLIT):
        rows = pl.ds(pl.multiple_of(step * TF + b * R, R), R)
        h1s.append(x_s[rows, :].astype(F32) + _dot(pltpu.bitcast(on_s[pl.ds(b * R // 2, R // 2), :], BF16), wo_s[...]))
    stage_attn(jnp.minimum(step + 1, S // TF - 1))
    for b in range(FSPLIT):
        hn = _layernorm(h1s[b]).astype(BF16)
        if PIN and b == FSPLIT - 1:
            z = jnp.minimum(step, 0)
            tap = on_s[pl.ds(pl.multiple_of(z * 8, 8), 8), 0:128] & z.astype(U32)
            hp = pltpu.bitcast(hn, U32)
            top = jnp.concatenate([hp[0:8, 0:128] | tap, hp[0:8, 128:]], axis=1)
            hn = pltpu.bitcast(jnp.concatenate([top, hp[8:]], axis=0), BF16)
        if FFN_T:
            act = _gelu_tanh(_dot_nt(wg_s[...], hn)) * _dot_nt(wu_s[...], hn)
            acts.append(act.astype(BF16).T if FFN_T == 1 else act.T.astype(BF16))
        else:
            acts.append(
                (_gelu_tanh(_dot_nt(hn, wg_s[...])) * _dot_nt(hn, wu_s[...])).astype(BF16))
    def out_copy(r0, i):
        rows = pl.ds(r0, R)
        return pltpu.make_async_copy(ob_s.at[rows], o_ref.at[rows], osems.at[i])

    for b in range(FSPLIT):
        r0 = pl.multiple_of(step * TF + b * R, R)
        ob_s[pl.ds(r0, R), :] = (h1s[b] + _dot(acts[b], wd_s[...])).astype(ob_s.dtype)
        out_copy(r0, step * FSPLIT + b).start()

    @pl.when(step == S // TF - 1)
    def _():
        for i in range(S // R):
            out_copy(i * R, i).wait()


@jax.jit
def pallas_sequential_preLN__softmax_full_mha__geglu_ffn__prompt_kernel(
    A_x: jax.Array,
    A_wqkv: jax.Array,
    A_wo: jax.Array,
    B_x: jax.Array,
    B_w_gate: jax.Array,
    B_w_up: jax.Array,
    B_w_down: jax.Array,
):
    B, S, D = A_x.shape
    F = B_w_gate.shape[1]
    assert B == 1 and D == H * DH and sum(CHUNKS) == S and TF % TQ == 0
    x = A_x.reshape(S, D)
    G = D // 128
    NC = S // TK
    hbm = pl.BlockSpec(memory_space=pltpu.MemorySpace.HBM)
    nvmax = 8 * max(NVP)
    packed_rows = max(PADR, 4 * sum(TK // 8 - NVP[c % len(NVP)] for c in range(NC)))

    out = pl.pallas_call(
        functools.partial(_kernel, S=S, D=D),
        grid=(S // TF,),
        in_specs=[hbm] * 6,
        out_specs=hbm,
        out_shape=jax.ShapeDtypeStruct((S, D), A_x.dtype),
        scratch_shapes=[
            pltpu.VMEM((S, D), BF16),
            pltpu.VMEM((3, D, D), BF16),
            pltpu.VMEM((G, S, 128), F32),
            pltpu.VMEM((G, packed_rows, 128), U32),
            pltpu.VMEM((H, DH, S), F32),
            pltpu.VMEM((H, DH, S), F32),
            pltpu.VMEM((packed_rows, 128), U32),
            pltpu.VMEM((packed_rows, 128), U32),
            pltpu.VMEM((NC, DH, nvmax, 128), F32),
            pltpu.VMEM((NC, DH, nvmax, 128), F32),
            pltpu.VMEM((S, 128), F32),
            pltpu.VMEM((NC, TK, TQ), F32),
            pltpu.VMEM((TK, TQ), F32),
            pltpu.VMEM((S // TF, H, DH, TF), F32),
            pltpu.VMEM((S // 128, H * 8, 128), F32),
            pltpu.VMEM((H, TF), F32),
            pltpu.VMEM((TF // 2, D), U32),
            pltpu.VMEM((S, D), A_x.dtype),
            pltpu.VMEM((D, D), BF16),
            pltpu.VMEM((F, D), BF16),
            pltpu.VMEM((F, D), BF16),
            pltpu.VMEM((F, D), BF16),
            pltpu.SemaphoreType.DMA((11,)),
            pltpu.SemaphoreType.DMA((S // TF * FSPLIT,)),
        ],
        compiler_params=pltpu.CompilerParams(
            dimension_semantics=("arbitrary",),
            vmem_limit_bytes=100 * 1024 * 1024,
        ),
    )(x, A_wqkv, A_wo, B_w_gate.T, B_w_up.T, B_w_down)
    return out.reshape(B, S, D)
```

```python
import functools
import math

import jax
import jax.numpy as jnp
import jax.experimental.pallas as pl
import jax.experimental.pallas.tpu as pltpu

H = 32
DH = 16
HPG = 128 // DH
EPS = 1e-5
TQ = 512
TK = 128
TS = 512
FSPLIT = 2
CHUNKS = (256, 256, 512, 512, 512)
NVP = (3, 3, 3, 3, 2, 3, 3, 2, 3, 3, 2, 3, 3, 2, 3, 3)
LEAD = 3
VOFF = 3
FILL0 = 2
FILL1 = 60
SUM_LIMIT = 2.0 ** 64
VALUE_LIMIT = 2.0 ** 30

F32 = jnp.float32
BF16 = jnp.bfloat16
U32 = jnp.uint32


def _layernorm(x):
    m = jnp.mean(x, axis=-1, keepdims=True)
    d = x - m
    v = jnp.mean(d * d, axis=-1, keepdims=True)
    return d * jax.lax.rsqrt(v + EPS)


def _gelu_tanh(x):
    c = math.sqrt(2.0 / math.pi)
    return 0.5 * x * (1.0 + jnp.tanh(c * (x + 0.044715 * (x * x * x))))


def _dot(a, b):
    return jnp.dot(a, b, preferred_element_type=F32)


def _dot_nt(a, b):
    return jax.lax.dot_general(a, b, (((1,), (1,)), ((), ())),
                               preferred_element_type=F32)


def _pack(x):
    return pltpu.bitcast(x, U32)


def _unpack(x):
    return pltpu.bitcast(x, BF16)


def _rows_max8(x):
    return jnp.max(x.reshape(x.shape[0] // 8, 8, x.shape[1]), axis=0)


def _abs_max8(x):
    a = jnp.abs(x)
    m = a[:, 0:128]
    for g in range(1, x.shape[1] // 128):
        m = jnp.maximum(m, a[:, g * 128:(g + 1) * 128])
    return _rows_max8(m)


def _lane_gather(x, idx8):
    idx = jnp.concatenate([idx8] * (x.shape[0] // 8), axis=0)
    return jnp.take_along_axis(x, idx, axis=1, mode="promise_in_bounds")


def _lane_shift(x, n):
    lane = jax.lax.broadcasted_iota(jnp.int32, (8, 128), 1)
    return _lane_gather(x, (lane + n) & 127)


def _lane_splat(x, n):
    return _lane_gather(x, jnp.zeros((8, 128), jnp.int32) + n)


def _kernel(x_hbm, wqkv_hbm, wo_hbm, wg_hbm, wu_hbm, wd_hbm, o_hbm,
            x_s, wqkv_s, k_s, kp_s, qt_s, vt_s, kh0, kh1, kb0, kb1,
            kf_s, sc_s, pend_s, ot_s, l_s, r_s, on_s, ob_s,
            wo_s, wg_s, wu_s, wd_s, sems, osems, *, S, D):
    step = pl.program_id(0)
    G = D // 128
    NC = S // TK
    NT = S // TQ
    NG = TK // 8
    NJ = TQ // 128
    R = TQ // FSPLIT
    q_scale = (DH ** -0.5) * math.log2(math.e)
    nv = [NVP[c % len(NVP)] for c in range(NC)]
    starts = [sum(CHUNKS[:i]) for i in range(len(CHUNKS))]
    order = [(c, g) for c in range(NC) for g in reversed(range(nv[c], NG))]
    first = [sum(NG - nv[i] for i in range(c)) for c in range(NC + 1)]
    NS = len(order)
    assert NS % 2 == 0
    khs, tabs = (kh0, kh1), (kb0, kb1)

    x_parts = [(starts[i], CHUNKS[i]) for i in range(3)] + [(starts[3], S - starts[3])]
    x_copies = [
        pltpu.make_async_copy(x_hbm.at[pl.ds(r0, n)], x_s.at[pl.ds(r0, n)], sems.at[i])
        for i, (r0, n) in enumerate(x_parts)]
    wq_copy, wk_copy, wv_copy = [
        pltpu.make_async_copy(wqkv_hbm.at[:, pl.ds(i * D, D)], wqkv_s.at[i], sems.at[4 + i])
        for i in range(3)]
    late_copies = [
        pltpu.make_async_copy(src, dst, sems.at[7 + i])
        for i, (src, dst) in enumerate(
            [(wo_hbm, wo_s), (wg_hbm, wg_s), (wu_hbm, wu_s), (wd_hbm, wd_s)])
    ]

    def norm_rows(ci):
        return _layernorm(x_s[pl.ds(starts[ci], CHUNKS[ci]), :].astype(F32)).astype(BF16)

    def project_k(ci, xn):
        r0, n = starts[ci], CHUNKS[ci]
        c0, c1 = r0 // TK, (r0 + n) // TK
        k = _dot(xn, wqkv_s[1])
        kp = jnp.concatenate(
            [k[(c - c0) * TK + 8 * g:(c - c0) * TK + 8 * g + 8]
             for c, g in order[first[c0]:first[c1]]], axis=0)
        kp = _pack(kp.astype(BF16))
        prows = pl.ds(first[c0] * 4, (first[c1] - first[c0]) * 4)
        for g in range(G):
            k_s[g, pl.ds(r0, n), :] = k[:, g * 128:(g + 1) * 128]
            kp_s[g, prows, :] = kp[:, g * 128:(g + 1) * 128]
        kh0[prows, :] = kp[:, 0:128]
        for c in range(c0, c1):
            rows = k[(c - c0) * TK:(c - c0) * TK + 8 * nv[c], 0:128]
            for d in range(DH):
                kb0[c, d, 0:8 * nv[c], :] = _lane_splat(rows, d)

    def project_q(ci, xn):
        q = _dot(xn, wqkv_s[0]) * q_scale
        qt_s[:, :, pl.ds(starts[ci], CHUNKS[ci])] = q.T.reshape(H, DH, CHUNKS[ci])

    def project_v(ci, xn):
        v = _dot(xn, wqkv_s[2])
        vt_s[:, :, pl.ds(starts[ci], CHUNKS[ci])] = v.T.reshape(H, DH, CHUNKS[ci])

    def store_sums(h, qi, cols):
        for j in range(NJ):
            l_s[qi * NJ + j, pl.ds(pl.multiple_of(h * 8, 8), 8), :] = cols[j]

    def vpu_scores(h, qi, c, j, kb, z):
        accs = [None] * nv[c]
        for d in range(DH):
            qb = jnp.broadcast_to(
                qt_s[h, d:d + 1, pl.ds(qi * TQ + j * 128, 128)], (8, 128))
            for g in range(nv[c]):
                t = kb[c + z, d, 8 * g:8 * (g + 1), :] * qb
                accs[g] = t if accs[g] is None else accs[g] + t
        return accs

    def prep_piece(h, pc, kh, kb):
        g, lane0 = h // HPG, (h % HPG) * DH
        if pc % 8 == 0:
            i, n = pc // 8, 4 * DH // 8
            lo, hi = (i * (NS // 2)) // n, ((i + 1) * (NS // 2)) // n
            rows = pl.ds(8 * lo, 8 * (hi - lo))
            kh[rows, :] = _lane_shift(kp_s[g, rows, :], lane0)
        d, part = divmod(pc, 4)
        for c in range(part * (NC // 4), (part + 1) * (NC // 4)):
            kb[c, d, 0:8 * nv[c], :] = _lane_splat(
                k_s[g, pl.ds(c * TK, 8 * nv[c]), :], lane0 + d)

    def finish_pending(h, acc, top):
        n = 8 * nv[NC - 1]
        pt = jnp.concatenate([top, pend_s[pl.ds(n, TK - n), :]], axis=0)
        ot_s[NT - 1, h] = acc + _dot(vt_s[h, :, pl.ds((NC - 1) * TK, TK)], pt)

    def head_pair(jj, carry):
        lmin, lmax, acc_prev, top_prev = carry
        h0 = 2 * jj
        zs = [jnp.minimum(jj, 0) * (j + 1) for j in range(NJ)]
        zero = zs[0].astype(F32)
        units = [(hh, qi) for hh in range(2) for qi in range(NT)]
        total = len(units) * NC
        slen = len(units) * NS
        ends = [(t // NC) * NS + first[t % NC + 1] for t in range(total)]
        cuts = [min(e + LEAD + (e + LEAD) % 2, slen) for e in ends]
        pieces = {}
        work = sum(nv) * NJ * len(units)
        done = 0
        for t in range(total):
            for j in range(NJ):
                pos = min((done * slen) // work + VOFF, cuts[t] - 1)
                if t == total - 1:
                    pos = slen - 1
                pieces.setdefault(pos, []).append((t, j))
                done += nv[t % NC]
        probs = {}
        lacc = {}
        qhs = {}
        acc = None

        def consume(t, g, j, sg):
            p = jnp.exp2(sg)
            key = (t // NC, j)
            lacc[key] = p if key not in lacc else lacc[key] + p
            probs[(t, g, j)] = p

        def score_rows(lo, hi):
            ui = lo // NS
            hh, qi = units[ui]
            if ui not in qhs:
                qhs[ui] = qt_s[h0 + hh, :, pl.ds(qi * TQ, TQ)].astype(BF16)
            kk = _unpack(khs[hh][pl.ds(4 * (lo - ui * NS), 4 * (hi - lo)), :])
            s = _dot(kk[:, 0:DH], qhs[ui])
            for i in range(lo, hi):
                for tv, j in pieces.get(i, ()):
                    hv, qv = units[tv // NC]
                    sv = vpu_scores(h0 + hv, qv, tv % NC, j, tabs[hv], zs[j])
                    for gv in reversed(range(len(sv))):
                        consume(tv, gv, j, sv[gv])
                c, g = order[i - ui * NS]
                r = 8 * (i - lo)
                for j in range(NJ):
                    consume(ui * NC + c, g, j, s[r:r + 8, 128 * j:128 * (j + 1)])

        lo = 0
        for t in range(total + 1):
            if t < total:
                hi = cuts[t]
                cut = min(hi, (lo // NS + 1) * NS)
                if cut > lo:
                    score_rows(lo, cut)
                if hi > cut:
                    score_rows(cut, hi)
                lo = hi
                hh, qi = units[t // NC]
                hn = jnp.minimum(h0 + hh + 1, H - 1)
                for pc in range(4 * DH):
                    if FILL0 + (pc * (FILL1 - FILL0)) // (4 * DH) == qi * NC + t % NC:
                        prep_piece(hn, pc, khs[1 - hh], tabs[1 - hh])
            if t == 0:
                finish_pending(jnp.maximum(h0 - 1, 0), acc_prev, top_prev)
                continue
            u = t - 1
            ui, c = divmod(u, NC)
            hh, qi = units[ui]
            h = h0 + hh
            pt = jnp.concatenate(
                [jnp.concatenate([probs.pop((u, g, j)) for j in range(NJ)], axis=1)
                 for g in range(NG)], axis=0)
            if c == NC - 1:
                for j in range(NJ):
                    lmin = jnp.minimum(lmin, lacc[ui, j])
                    lmax = jnp.maximum(lmax, lacc[ui, j])
                store_sums(h, qi, [lacc[ui, j] for j in range(NJ)])
            if u == total - 1:
                n = 8 * nv[c]
                pend_s[pl.ds(n, TK - n), :] = pt[n:]
                return lmin, lmax, acc, pt[0:n]
            acc = (zero if c == 0 else acc) + _dot(vt_s[h, :, pl.ds(c * TK, TK)], pt)
            if c == NC - 1:
                ot_s[qi, h] = acc

    def safe_head(h, carry):
        def shift_keys(c, carry):
            rows = pl.ds(pl.multiple_of(c * TK, TK), TK)
            kf_s[rows, :] = _lane_shift(k_s[h // HPG, rows, :], (h % HPG) * DH)
            return carry

        jax.lax.fori_loop(0, NC, shift_keys, 0)

        def tile(qi, carry):
            qh = qt_s[h, :, pl.ds(pl.multiple_of(qi * TQ, TQ), TQ)]

            def scores(c, m8):
                s = _dot(kf_s[pl.ds(pl.multiple_of(c * TS, TS), TS), :][:, 0:DH], qh)
                sc_s[c] = s
                return jnp.maximum(m8, _rows_max8(s))

            m8 = jax.lax.fori_loop(0, S // TS, scores, jnp.full((8, TQ), -jnp.inf, F32))
            m = jnp.max(m8, axis=0, keepdims=True)

            def weigh(c, st):
                acc, l8 = st
                p = jnp.exp2(sc_s[c] - m)
                v = vt_s[h, :, pl.ds(pl.multiple_of(c * TS, TS), TS)]
                return (acc + _dot(v, p),
                        l8 + jnp.sum(p.reshape(TS // 8, 8, TQ), axis=0))

            acc, l8 = jax.lax.fori_loop(
                0, S // TS, weigh, (jnp.zeros((DH, TQ), F32), jnp.zeros((8, TQ), F32)))
            ot_s[qi, h] = acc
            store_sums(h, qi, [l8[:, 128 * j:128 * (j + 1)] for j in range(NJ)])
            return carry

        return jax.lax.fori_loop(0, NT, tile, carry)

    def attn_rows(blk, b):
        js = range(b * R // 128, (b + 1) * R // 128)
        for j in js:
            l = l_s[blk * NJ + j, pl.ds(0, H, stride=8), :]
            for i in range(1, 8):
                l = l + l_s[blk * NJ + j, pl.ds(i, H, stride=8), :]
            r_s[:, 128 * j:128 * (j + 1)] = 1.0 / l
        heads = []
        for h in range(H):
            r = jnp.concatenate(
                [jnp.broadcast_to(r_s[h:h + 1, 128 * j:128 * (j + 1)], (8, 128))
                 for j in js], axis=1)
            heads.append(ot_s[blk, h, :, pl.ds(b * R, R)] * jnp.concatenate([r, r], axis=0))
        return jnp.concatenate(heads, axis=0).T.astype(BF16)

    def stage_attn(blk):
        on_s[...] = _pack(attn_rows(blk, 0))

    @pl.when(step == 0)
    def _():
        for cp in (x_copies[0], wk_copy, x_copies[1], wq_copy, wv_copy,
                   x_copies[2], x_copies[3]):
            cp.start()
        pend_s[...] = jnp.zeros(pend_s.shape, F32)
        x_copies[0].wait()
        xn0 = norm_rows(0)
        wk_copy.wait()
        project_k(0, xn0)
        x_copies[1].wait()
        wq_copy.wait()
        project_q(0, xn0)
        xn1 = norm_rows(1)
        project_q(1, xn1)
        project_k(1, xn1)
        wv_copy.wait()
        x_copies[2].wait()
        project_v(0, xn0)
        project_v(1, xn1)
        wv8 = _abs_max8(wqkv_s[2].astype(F32))
        xn = norm_rows(2)
        project_v(2, xn)
        project_k(2, xn)
        x_copies[3].wait()
        for cp in late_copies:
            cp.start()
        project_q(2, xn)
        for ci in range(3, len(CHUNKS)):
            xn = norm_rows(ci)
            project_v(ci, xn)
            project_q(ci, xn)
            project_k(ci, xn)

        ones = jnp.ones((8, 128), F32)
        lmin, lmax, acc, top = jax.lax.fori_loop(
            0, H // 2, head_pair,
            (ones, ones, jnp.zeros((DH, TQ), F32), jnp.zeros((8 * nv[NC - 1], TQ), F32)))
        finish_pending(H - 1, acc, top)
        stage_attn(0)
        worst = jnp.max(jnp.maximum(jnp.maximum(lmax, 1.0 / lmin) * (1.0 / SUM_LIMIT),
                                    wv8 * (D / VALUE_LIMIT)))

        @pl.when(jnp.logical_not(worst <= 1.0))
        def _():
            jax.lax.fori_loop(0, H, safe_head, 0)
            stage_attn(0)

        for cp in late_copies:
            cp.wait()

    h1s, acts = [], []
    for b in range(FSPLIT):
        rows = pl.ds(pl.multiple_of(step * TQ + b * R, R), R)
        o = _unpack(on_s[...]) if b == 0 else attn_rows(step, b)
        h1s.append(x_s[rows, :].astype(F32) + _dot(o, wo_s[...]))
    stage_attn(jnp.minimum(step + 1, NT - 1))
    for b in range(FSPLIT):
        hn = _layernorm(h1s[b]).astype(BF16)
        if b == FSPLIT - 1:
            z = jnp.minimum(step, 0)
            tap = on_s[pl.ds(pl.multiple_of(z * 8, 8), 8), 0:128] & z.astype(U32)
            hp = _pack(hn)
            top = jnp.concatenate([hp[0:8, 0:128] | tap, hp[0:8, 128:]], axis=1)
            hn = _unpack(jnp.concatenate([top, hp[8:]], axis=0))
        act = _gelu_tanh(_dot_nt(wg_s[...], hn)) * _dot_nt(wu_s[...], hn)
        acts.append(act.astype(BF16).T)

    def out_copy(r0, i):
        rows = pl.ds(r0, R)
        return pltpu.make_async_copy(ob_s.at[rows], o_hbm.at[rows], osems.at[i])

    for b in range(FSPLIT):
        r0 = pl.multiple_of(step * TQ + b * R, R)
        ob_s[pl.ds(r0, R), :] = (h1s[b] + _dot(acts[b], wd_s[...])).astype(ob_s.dtype)
        out_copy(r0, step * FSPLIT + b).start()

    @pl.when(step == NT - 1)
    def _():
        for i in range(S // R):
            out_copy(i * R, i).wait()


@jax.jit
def pallas_sequential_preLN__softmax_full_mha__geglu_ffn__prompt_kernel(
    A_x: jax.Array,
    A_wqkv: jax.Array,
    A_wo: jax.Array,
    B_x: jax.Array,
    B_w_gate: jax.Array,
    B_w_up: jax.Array,
    B_w_down: jax.Array,
):
    B, S, D = A_x.shape
    F = B_w_gate.shape[1]
    assert B == 1 and D == H * DH and sum(CHUNKS) == S
    G = D // 128
    NC = S // TK
    NT = S // TQ
    hbm = pl.BlockSpec(memory_space=pltpu.MemorySpace.HBM)

    out = pl.pallas_call(
        functools.partial(_kernel, S=S, D=D),
        grid=(NT,),
        in_specs=[hbm] * 6,
        out_specs=hbm,
        out_shape=jax.ShapeDtypeStruct((S, D), A_x.dtype),
        scratch_shapes=[
            pltpu.VMEM((S, D), BF16),
            pltpu.VMEM((3, D, D), BF16),
            pltpu.VMEM((G, S, 128), F32),
            pltpu.VMEM((G, S // 2, 128), U32),
            pltpu.VMEM((H, DH, S), F32),
            pltpu.VMEM((H, DH, S), F32),
            pltpu.VMEM((S // 2, 128), U32),
            pltpu.VMEM((S // 2, 128), U32),
            pltpu.VMEM((NC, DH, 8 * max(NVP), 128), F32),
            pltpu.VMEM((NC, DH, 8 * max(NVP), 128), F32),
            pltpu.VMEM((S, 128), F32),
            pltpu.VMEM((S // TS, TS, TQ), F32),
            pltpu.VMEM((TK, TQ), F32),
            pltpu.VMEM((NT, H, DH, TQ), F32),
            pltpu.VMEM((S // 128, H * 8, 128), F32),
            pltpu.VMEM((H, TQ), F32),
            pltpu.VMEM((TQ // FSPLIT // 2, D), U32),
            pltpu.VMEM((S, D), A_x.dtype),
            pltpu.VMEM((D, D), BF16),
            pltpu.VMEM((F, D), BF16),
            pltpu.VMEM((F, D), BF16),
            pltpu.VMEM((F, D), BF16),
            pltpu.SemaphoreType.DMA((11,)),
            pltpu.SemaphoreType.DMA((NT * FSPLIT,)),
        ],
        compiler_params=pltpu.CompilerParams(
            dimension_semantics=("arbitrary",),
            vmem_limit_bytes=100 * 1024 * 1024,
        ),
    )(A_x.reshape(S, D), A_wqkv, A_wo, B_w_gate.T, B_w_up.T, B_w_down)
    return out.reshape(B, S, D)
```

```python
import functools
import math

import jax
import jax.numpy as jnp
import jax.experimental.pallas as pl
import jax.experimental.pallas.tpu as pltpu

H = 32
DH = 16
HPG = 128 // DH
EPS = 1e-5
TQ = 512
TK = 128
TS = 512
FSPLIT = 2
CHUNKS = (256, 256, 512, 512, 512)
NVP = (3, 3, 2, 3)
LEAD = 3
VOFF = 3
FILL0 = 2
FILL1 = 60
SLAB = 16
GU_ORDER = (0, 6, 3, 4, 2, 1, 5)
DOWN_ORDER = (1, 3, 2, 4, 0, 6, 5)
SUM_LIMIT = 2.0 ** 64
VALUE_LIMIT = 2.0 ** 30

F32 = jnp.float32
BF16 = jnp.bfloat16
U32 = jnp.uint32


def _layernorm(x):
    m = jnp.mean(x, axis=-1, keepdims=True)
    d = x - m
    v = jnp.mean(d * d, axis=-1, keepdims=True)
    return d * jax.lax.rsqrt(v + EPS)


def _gelu_tanh(x):
    c = math.sqrt(2.0 / math.pi)
    return 0.5 * x * (1.0 + jnp.tanh(c * (x + 0.044715 * (x * x * x))))


def _dot(a, b):
    return jnp.dot(a, b, preferred_element_type=F32)


def _dot_nt(a, b):
    return jax.lax.dot_general(a, b, (((1,), (1,)), ((), ())),
                               preferred_element_type=F32)


def _quads(x):
    m, n = x.shape[0] // 2, x.shape[1] // 2
    return x[:m, :n], x[:m, n:], x[m:, :n], x[m:, n:]


def _strassen_left(a11, a12, a21, a22):
    return [a11 + a22, a21 + a22, a11, a22, a11 + a12, a21 - a11, a12 - a22]


def _strassen_right(b11, b12, b21, b22):
    return [b11 + b22, b11, b12 - b22, b21 - b11, b22, b11 + b12, b21 + b22]


def _strassen_combine(m):
    top = jnp.concatenate([m[0] + m[3] - m[4] + m[6], m[2] + m[4]], axis=1)
    bot = jnp.concatenate([m[1] + m[3], m[0] - m[1] + m[2] + m[5]], axis=1)
    return jnp.concatenate([top, bot], axis=0)


def _pack(x):
    return pltpu.bitcast(x, U32)


def _unpack(x):
    return pltpu.bitcast(x, BF16)


def _rows_max8(x):
    return jnp.max(x.reshape(x.shape[0] // 8, 8, x.shape[1]), axis=0)


def _abs_max8(x):
    a = jnp.abs(x)
    m = a[:, 0:128]
    for g in range(1, x.shape[1] // 128):
        m = jnp.maximum(m, a[:, g * 128:(g + 1) * 128])
    return _rows_max8(m)


def _lane_gather(x, idx):
    return jnp.take_along_axis(x, idx, axis=1, mode="promise_in_bounds")


def _lane_shift(x, n):
    lane = jax.lax.broadcasted_iota(jnp.int32, x.shape, 1)
    return _lane_gather(x, (lane + n) & 127)


def _lane_splat(x, n):
    return _lane_gather(x, jnp.full(x.shape, n, jnp.int32))


def _kernel(x_hbm, wqkv_hbm, wo_hbm, wg_hbm, wu_hbm, wd_hbm, o_hbm,
            x_s, wqkv_s, k_s, kp_s, qt_s, vt_s, kh0, kh1, kb0, kb1,
            kf_s, sc_s, pend_s, ot_s, l_s, r_s, on_s, ob_s,
            wo_s, wg_s, wu_s, wd_s, sg_s, su_s, sd_s, sems, osems, *, S, D, F):
    step = pl.program_id(0)
    G = D // 128
    NC = S // TK
    NT = S // TQ
    NG = TK // 8
    NJ = TQ // 128
    R = TQ // FSPLIT
    q_scale = (DH ** -0.5) * math.log2(math.e)
    nv = [NVP[c % len(NVP)] for c in range(NC)]
    starts = [sum(CHUNKS[:i]) for i in range(len(CHUNKS))]
    order = [(c, g) for c in range(NC) for g in reversed(range(nv[c], NG))]
    first = [sum(NG - nv[i] for i in range(c)) for c in range(NC + 1)]
    NS = len(order)
    assert NS % 2 == 0
    khs, tabs = (kh0, kh1), (kb0, kb1)

    x_parts = [(starts[i], CHUNKS[i]) for i in range(3)] + [(starts[3], S - starts[3])]
    x_copies = [
        pltpu.make_async_copy(x_hbm.at[pl.ds(r0, n)], x_s.at[pl.ds(r0, n)], sems.at[i])
        for i, (r0, n) in enumerate(x_parts)]
    wq_copy, wk_copy, wv_copy = [
        pltpu.make_async_copy(wqkv_hbm.at[:, pl.ds(i * D, D)], wqkv_s.at[i], sems.at[4 + i])
        for i in range(3)]
    late_copies = [
        pltpu.make_async_copy(src, dst, sems.at[7 + i])
        for i, (src, dst) in enumerate(
            [(wg_hbm, wg_s.at[pl.ds(0, F)]), (wu_hbm, wu_s.at[pl.ds(0, F)]),
             (wd_hbm, wd_s.at[pl.ds(0, F)]), (wo_hbm, wo_s)])
    ]

    def norm_rows(ci):
        return _layernorm(x_s[pl.ds(starts[ci], CHUNKS[ci]), :].astype(F32)).astype(BF16)

    def project_k(ci, xn):
        r0, n = starts[ci], CHUNKS[ci]
        c0, c1 = r0 // TK, (r0 + n) // TK
        k = _dot(xn, wqkv_s[1])
        kp = jnp.concatenate(
            [k[(c - c0) * TK + 8 * g:(c - c0) * TK + 8 * g + 8]
             for c, g in order[first[c0]:first[c1]]], axis=0)
        kp = _pack(kp.astype(BF16))
        prows = pl.ds(first[c0] * 4, (first[c1] - first[c0]) * 4)
        for g in range(G):
            k_s[g, pl.ds(r0, n), :] = k[:, g * 128:(g + 1) * 128]
            kp_s[g, prows, :] = kp[:, g * 128:(g + 1) * 128]
        kh0[prows, :] = kp[:, 0:128]
        for c in range(c0, c1):
            rows = k[(c - c0) * TK:(c - c0) * TK + 8 * nv[c], 0:128]
            for d in range(DH):
                kb0[c, d, 0:8 * nv[c], :] = _lane_splat(rows, d)

    def project_q(ci, xn):
        q = _dot(xn, wqkv_s[0]) * q_scale
        qt_s[:, :, pl.ds(starts[ci], CHUNKS[ci])] = q.T.reshape(H, DH, CHUNKS[ci])
        return q

    def project_v(ci, xn):
        v = _dot(xn, wqkv_s[2])
        vt_s[:, :, pl.ds(starts[ci], CHUNKS[ci])] = v.T.reshape(H, DH, CHUNKS[ci])
        return v

    def store_sums(h, qi, cols):
        for j in range(NJ):
            l_s[qi * NJ + j, pl.ds(pl.multiple_of(h * 8, 8), 8), :] = cols[j]

    KD = (F // 256) * 256

    def weight_sums(src, dst, rows, operands, pace):
        m, n = rows // 2, D // 2
        z = jnp.minimum(step, 0)
        slabs = m // SLAB
        per = -(-slabs // G)
        for i in range(slabs):
            g, r = divmod(i, per)
            r = (r * (pace.shape[0] // 16) // per) * 16
            src[pl.ds(F, 16), 0:128] = pace[r:r + 16, 128 * g:128 * (g + 1)].astype(BF16)
            rs = [pl.ds(pl.multiple_of(z + (r0 + i * SLAB), SLAB), SLAB) for r0 in (0, m)]
            quads = [src[r, pl.ds(c0, n)].astype(F32) for r in rs for c0 in (0, n)]
            sums = [t for t in operands(*quads) if not any(t is q for q in quads)]
            for j, t in enumerate(sums):
                dst[j, pl.ds(i * SLAB, SLAB), :] = t.astype(BF16)

    def weight_operands(src, dst, rows, plain):
        m, n = rows // 2, D // 2
        out, i = [], 0
        for j in range(7):
            if j in plain:
                r0, c0 = plain[j]
                out.append(src[pl.ds(r0 * m, m), pl.ds(c0 * n, n)])
            else:
                out.append(dst[i, pl.ds(0, m), :])
                i += 1
        return out

    def vpu_scores(h, qi, c, j, kb, z):
        n = 8 * nv[c]
        cz = c + z
        cols = pl.ds(qi * TQ + j * 128, 128)
        acc = None
        for d in range(DH):
            t = kb[cz, d, 0:n, :] * qt_s[h, d:d + 1, cols]
            acc = t if acc is None else acc + t
        return acc

    def prep_piece(g, lane0, pc, kh, kb):
        if pc % 8 == 0:
            i, n = pc // 8, 4 * DH // 8
            lo, hi = (i * (NS // 2)) // n, ((i + 1) * (NS // 2)) // n
            rows = pl.ds(8 * lo, 8 * (hi - lo))
            kh[rows, :] = _lane_shift(kp_s[g, rows, :], lane0)
        d, part = divmod(pc, 4)
        cs = range(part * (NC // 4), (part + 1) * (NC // 4))
        col = _lane_splat(jnp.concatenate(
            [k_s[g, pl.ds(c * TK, 8 * nv[c]), :] for c in cs], axis=0), lane0 + d)
        r = 0
        for c in cs:
            kb[c, d, 0:8 * nv[c], :] = col[r:r + 8 * nv[c]]
            r += 8 * nv[c]

    def finish_pending(h, acc, top):
        n = 8 * nv[NC - 1]
        pt = jnp.concatenate([top, pend_s[pl.ds(n, TK - n), :]], axis=0)
        ot_s[NT - 1, h] = acc + _dot(vt_s[h, :, pl.ds((NC - 1) * TK, TK)], pt)

    def head_pair(jj, carry):
        lmin, lmax, acc_prev, top_prev = carry
        hs = (2 * jj, 2 * jj + 1)
        nxt = [jnp.minimum(h + 1, H - 1) for h in hs]
        nxt = [(h // HPG, (h % HPG) * DH) for h in nxt]
        zs = [jnp.minimum(jj, 0) * (j + 1) for j in range(NJ)]
        zero = zs[0].astype(F32)
        units = [(hh, qi) for hh in range(2) for qi in range(NT)]
        total = len(units) * NC
        slen = len(units) * NS
        ends = [(t // NC) * NS + first[t % NC + 1] for t in range(total)]
        cuts = [min(e + LEAD + (e + LEAD) % 2, slen) for e in ends]
        pieces = {}
        work = sum(nv) * NJ * len(units)
        done = 0
        for t in range(total):
            for j in range(NJ):
                pos = min((done * slen) // work + VOFF, cuts[t] - 1)
                if t == total - 1:
                    pos = slen - 1
                pieces.setdefault(pos, []).append((t, j))
                done += nv[t % NC]
        mxu_p = {}
        vpu_p = {}
        lacc = {}
        qhs = {}
        acc = None

        def add_sums(ui, js, p):
            if all((ui, j) in lacc for j in js):
                prev = [lacc[ui, j] for j in js]
                prev = prev[0] if len(js) == 1 else jnp.concatenate(prev, axis=1)
                p = jnp.concatenate([prev, p], axis=0)
                fresh = js
            else:
                fresh = [j for j in js if (ui, j) not in lacc]
            if p.shape[0] > 8:
                p = jnp.sum(p.reshape(p.shape[0] // 8, 8, p.shape[1]), axis=0)
            for i, j in enumerate(js):
                pj = p if len(js) == 1 else p[:, 128 * i:128 * (i + 1)]
                lacc[ui, j] = pj if j in fresh else lacc[ui, j] + pj

        def score_rows(lo, hi):
            ui = lo // NS
            hh, qi = units[ui]
            if ui not in qhs:
                qhs[ui] = qt_s[hs[hh], :, pl.ds(qi * TQ, TQ)].astype(BF16)
            kk = _unpack(khs[hh][pl.ds(4 * (lo - ui * NS), 4 * (hi - lo)), :])
            s = _dot(kk[:, 0:DH], qhs[ui])
            marks = sorted({lo, hi} | {i for i in pieces if lo < i < hi})
            for a, b in zip(marks[:-1], marks[1:]):
                for tv, j in pieces.get(a, ()):
                    hv, qv = units[tv // NC]
                    p = jnp.exp2(vpu_scores(hs[hv], qv, tv % NC, j, tabs[hv], zs[j]))
                    add_sums(tv // NC, [j], p)
                    vpu_p[tv, j] = p
                p = jnp.exp2(s[8 * (a - lo):8 * (b - lo)])
                add_sums(ui, list(range(NJ)), p)
                for i in range(a, b):
                    c, g = order[i - ui * NS]
                    mxu_p[ui * NC + c, g] = p[8 * (i - a):8 * (i - a + 1)]

        lo = 0
        for t in range(total + 1):
            if t < total:
                hi = cuts[t]
                cut = min(hi, (lo // NS + 1) * NS)
                if cut > lo:
                    score_rows(lo, cut)
                if hi > cut:
                    score_rows(cut, hi)
                lo = hi
                hh, qi = units[t // NC]
                for pc in range(4 * DH):
                    if FILL0 + (pc * (FILL1 - FILL0)) // (4 * DH) == qi * NC + t % NC:
                        prep_piece(*nxt[hh], pc, khs[1 - hh], tabs[1 - hh])
            if t == 0:
                finish_pending(jnp.maximum(hs[0] - 1, 0), acc_prev, top_prev)
                continue
            u = t - 1
            ui, c = divmod(u, NC)
            hh, qi = units[ui]
            h = hs[hh]
            top = jnp.concatenate([vpu_p.pop((u, j)) for j in range(NJ)], axis=1)
            rest = [mxu_p.pop((u, g)) for g in range(nv[c], NG)]
            if c == NC - 1:
                for j in range(NJ):
                    lmin = jnp.minimum(lmin, lacc[ui, j])
                    lmax = jnp.maximum(lmax, lacc[ui, j])
                store_sums(h, qi, [lacc[ui, j] for j in range(NJ)])
            if u == total - 1:
                pend_s[pl.ds(8 * nv[c], TK - 8 * nv[c]), :] = jnp.concatenate(rest, axis=0)
                return lmin, lmax, acc, top
            pt = jnp.concatenate([top] + rest, axis=0)
            acc = (zero if c == 0 else acc) + _dot(vt_s[h, :, pl.ds(c * TK, TK)], pt)
            if c == NC - 1:
                ot_s[qi, h] = acc

    def safe_head(h, carry):
        def shift_keys(c, carry):
            rows = pl.ds(pl.multiple_of(c * TK, TK), TK)
            kf_s[rows, :] = _lane_shift(k_s[h // HPG, rows, :], (h % HPG) * DH)
            return carry

        jax.lax.fori_loop(0, NC, shift_keys, 0)

        def tile(qi, carry):
            qh = qt_s[h, :, pl.ds(pl.multiple_of(qi * TQ, TQ), TQ)]

            def scores(c, m8):
                s = _dot(kf_s[pl.ds(pl.multiple_of(c * TS, TS), TS), :][:, 0:DH], qh)
                sc_s[c] = s
                return jnp.maximum(m8, _rows_max8(s))

            m8 = jax.lax.fori_loop(0, S // TS, scores, jnp.full((8, TQ), -jnp.inf, F32))
            m = jnp.max(m8, axis=0, keepdims=True)

            def weigh(c, st):
                acc, l8 = st
                p = jnp.exp2(sc_s[c] - m)
                v = vt_s[h, :, pl.ds(pl.multiple_of(c * TS, TS), TS)]
                return (acc + _dot(v, p),
                        l8 + jnp.sum(p.reshape(TS // 8, 8, TQ), axis=0))

            acc, l8 = jax.lax.fori_loop(
                0, S // TS, weigh, (jnp.zeros((DH, TQ), F32), jnp.zeros((8, TQ), F32)))
            ot_s[qi, h] = acc
            store_sums(h, qi, [l8[:, 128 * j:128 * (j + 1)] for j in range(NJ)])
            return carry

        return jax.lax.fori_loop(0, NT, tile, carry)

    def attn_rows(blk, b):
        js = range(b * R // 128, (b + 1) * R // 128)
        for j in js:
            l = l_s[blk * NJ + j, pl.ds(0, H, stride=8), :]
            for i in range(1, 8):
                l = l + l_s[blk * NJ + j, pl.ds(i, H, stride=8), :]
            r_s[:, 128 * j:128 * (j + 1)] = 1.0 / l
        heads = []
        for h in range(H):
            r = jnp.concatenate(
                [jnp.broadcast_to(r_s[h:h + 1, 128 * j:128 * (j + 1)], (8, 128))
                 for j in js], axis=1)
            heads.append(ot_s[blk, h, :, pl.ds(b * R, R)] * jnp.concatenate([r, r], axis=0))
        return jnp.concatenate(heads, axis=0).T.astype(BF16)

    def stage_attn(blk):
        on_s[...] = _pack(attn_rows(blk, 0))

    @pl.when(step == 0)
    def _():
        for cp in (x_copies[0], wk_copy, x_copies[1], wq_copy, wv_copy,
                   x_copies[2], x_copies[3], *late_copies):
            cp.start()
        pend_s[...] = jnp.zeros(pend_s.shape, F32)
        x_copies[0].wait()
        xn0 = norm_rows(0)
        wk_copy.wait()
        project_k(0, xn0)
        x_copies[1].wait()
        wq_copy.wait()
        project_q(0, xn0)
        xn1 = norm_rows(1)
        project_q(1, xn1)
        project_k(1, xn1)
        wv_copy.wait()
        x_copies[2].wait()
        project_v(0, xn0)
        project_v(1, xn1)
        wv8 = _abs_max8(wqkv_s[2].astype(F32))
        xn = norm_rows(2)
        project_v(2, xn)
        project_k(2, xn)
        x_copies[3].wait()
        project_q(2, xn)
        xn3 = norm_rows(3)
        project_v(3, xn3)
        xn4 = norm_rows(4)
        project_k(4, xn4)
        for cp in late_copies[:3]:
            cp.wait()
        weight_sums(wg_s, sg_s, F, _strassen_left, project_q(3, xn3))
        weight_sums(wu_s, su_s, F, _strassen_left, project_v(4, xn4))
        weight_sums(wd_s, sd_s, KD, _strassen_right, project_q(4, xn4))
        project_k(3, xn3)

        ones = jnp.ones((8, 128), F32)
        lmin, lmax, acc, top = jax.lax.fori_loop(
            0, H // 2, head_pair,
            (ones, ones, jnp.zeros((DH, TQ), F32), jnp.zeros((8 * nv[NC - 1], TQ), F32)))
        late_copies[3].wait()
        finish_pending(H - 1, acc, top)
        stage_attn(0)
        worst = jnp.max(jnp.maximum(jnp.maximum(lmax, 1.0 / lmin) * (1.0 / SUM_LIMIT),
                                    wv8 * (D / VALUE_LIMIT)))

        @pl.when(jnp.logical_not(worst <= 1.0))
        def _():
            jax.lax.fori_loop(0, H, safe_head, 0)
            stage_attn(0)

    h1s, acts = [], []
    for b in range(FSPLIT):
        rows = pl.ds(pl.multiple_of(step * TQ + b * R, R), R)
        o = _unpack(on_s[...]) if b == 0 else attn_rows(step, b)
        h1s.append(x_s[rows, :].astype(F32) + _dot(o, wo_s[...]))
    stage_attn(jnp.minimum(step + 1, NT - 1))
    for b in range(FSPLIT):
        hn = _layernorm(h1s[b])
        if b == FSPLIT - 1:
            z = jnp.minimum(step, 0)
            tap = on_s[pl.ds(pl.multiple_of(z * 8, 8), 8), 0:128] & z.astype(U32)
            hp = pltpu.bitcast(hn, U32)
            top = jnp.concatenate([hp[0:8, 0:128] | tap, hp[0:8, 128:]], axis=1)
            hn = pltpu.bitcast(jnp.concatenate([top, hp[8:]], axis=0), F32)
        t11, t21, t12, t22 = _quads(hn)
        ts = [t.astype(BF16) for t in _strassen_right(t11, t12, t21, t22)]
        ws = [weight_operands(src, dst, F, {2: (0, 0), 3: (1, 1)})
              for src, dst in ((wg_s, sg_s), (wu_s, su_s))]
        ms = [[None] * 7, [None] * 7]
        for i in GU_ORDER:
            for k in range(2):
                ms[k][i] = _dot_nt(ws[k][i], ts[i])
        acts.append(_gelu_tanh(_strassen_combine(ms[0])) * _strassen_combine(ms[1]))

    def down(act_t):
        a11, a21, a12, a22 = _quads(act_t[0:KD])
        ls = [a.astype(BF16).T for a in _strassen_left(a11, a12, a21, a22)]
        ws = weight_operands(wd_s, sd_s, KD, {1: (0, 0), 4: (1, 1)})
        tail = _dot(act_t[KD:].astype(BF16).T, wd_s[KD:F, :])
        ms = [None] * 7
        for i in DOWN_ORDER:
            ms[i] = _dot(ls[i], ws[i])
        return tail + _strassen_combine(ms)

    def out_copy(r0, i):
        rows = pl.ds(r0, R)
        return pltpu.make_async_copy(ob_s.at[rows], o_hbm.at[rows], osems.at[i])

    for b in range(FSPLIT):
        r0 = pl.multiple_of(step * TQ + b * R, R)
        ob_s[pl.ds(r0, R), :] = (h1s[b] + down(acts[b])).astype(ob_s.dtype)
        out_copy(r0, step * FSPLIT + b).start()

    @pl.when(step == NT - 1)
    def _():
        for i in range(S // R):
            out_copy(i * R, i).wait()


@jax.jit
def pallas_sequential_preLN__softmax_full_mha__geglu_ffn__prompt_kernel(
    A_x: jax.Array,
    A_wqkv: jax.Array,
    A_wo: jax.Array,
    B_x: jax.Array,
    B_w_gate: jax.Array,
    B_w_up: jax.Array,
    B_w_down: jax.Array,
):
    B, S, D = A_x.shape
    F = B_w_gate.shape[1]
    assert B == 1 and D == H * DH and sum(CHUNKS) == S
    G = D // 128
    NC = S // TK
    NT = S // TQ
    FP = -(-(F // 2) // 32) * 32
    hbm = pl.BlockSpec(memory_space=pltpu.MemorySpace.HBM)

    out = pl.pallas_call(
        functools.partial(_kernel, S=S, D=D, F=F),
        grid=(NT,),
        in_specs=[hbm] * 6,
        out_specs=hbm,
        out_shape=jax.ShapeDtypeStruct((S, D), A_x.dtype),
        scratch_shapes=[
            pltpu.VMEM((S, D), BF16),
            pltpu.VMEM((3, D, D), BF16),
            pltpu.VMEM((G, S, 128), F32),
            pltpu.VMEM((G, S // 2, 128), U32),
            pltpu.VMEM((H, DH, S), F32),
            pltpu.VMEM((H, DH, S), F32),
            pltpu.VMEM((S // 2, 128), U32),
            pltpu.VMEM((S // 2, 128), U32),
            pltpu.VMEM((NC, DH, 8 * max(NVP), 128), F32),
            pltpu.VMEM((NC, DH, 8 * max(NVP), 128), F32),
            pltpu.VMEM((S, 128), F32),
            pltpu.VMEM((S // TS, TS, TQ), F32),
            pltpu.VMEM((TK, TQ), F32),
            pltpu.VMEM((NT, H, DH, TQ), F32),
            pltpu.VMEM((S // 128, H * 8, 128), F32),
            pltpu.VMEM((H, TQ), F32),
            pltpu.VMEM((TQ // FSPLIT // 2, D), U32),
            pltpu.VMEM((S, D), A_x.dtype),
            pltpu.VMEM((D, D), BF16),
            pltpu.VMEM((F + 16, D), BF16),
            pltpu.VMEM((F + 16, D), BF16),
            pltpu.VMEM((F + 16, D), BF16),
            pltpu.VMEM((5, FP, D // 2), BF16),
            pltpu.VMEM((5, FP, D // 2), BF16),
            pltpu.VMEM((5, (F // 256) * 128, D // 2), BF16),
            pltpu.SemaphoreType.DMA((11,)),
            pltpu.SemaphoreType.DMA((NT * FSPLIT,)),
        ],
        compiler_params=pltpu.CompilerParams(
            dimension_semantics=("arbitrary",),
            vmem_limit_bytes=100 * 1024 * 1024,
        ),
    )(A_x.reshape(S, D), A_wqkv, A_wo, B_w_gate.T, B_w_up.T, B_w_down)
    return out.reshape(B, S, D)
```

```python
import functools
import math

import jax
import jax.numpy as jnp
import jax.experimental.pallas as pl
import jax.experimental.pallas.tpu as pltpu

H = 32
DH = 16
HPG = 128 // DH
EPS = 1e-5
TQ = 512
TK = 128
TS = 512
FSPLIT = 2
CHUNKS = (256, 256, 512, 512, 512)
NVP = (3, 2, 3, 3, 2, 3, 2, 3, 3, 2, 3, 2, 3, 3, 2, 3)
LEAD = 3
VOFF = 3
FILL0 = 2
FILL1 = 60
SLAB = 16
QKV_ORDER = (2, 3, 1, 4, 0, 6, 5)
GU_ORDER = (0, 6, 3, 4, 2, 1, 5)
DOWN_ORDER = (1, 3, 2, 4, 0, 6, 5)
SUM_LIMIT = 2.0 ** 64
VALUE_LIMIT = 2.0 ** 30

F32 = jnp.float32
BF16 = jnp.bfloat16
U32 = jnp.uint32


def _layernorm(x):
    m = jnp.mean(x, axis=-1, keepdims=True)
    d = x - m
    v = jnp.mean(d * d, axis=-1, keepdims=True)
    return d * jax.lax.rsqrt(v + EPS)


def _gelu_tanh(x):
    c = math.sqrt(2.0 / math.pi)
    return 0.5 * x * (1.0 + jnp.tanh(c * (x + 0.044715 * (x * x * x))))


def _dot(a, b):
    return jnp.dot(a, b, preferred_element_type=F32)


def _dot_nt(a, b):
    return jax.lax.dot_general(a, b, (((1,), (1,)), ((), ())),
                               preferred_element_type=F32)


def _quads(x):
    m, n = x.shape[0] // 2, x.shape[1] // 2
    return x[:m, :n], x[:m, n:], x[m:, :n], x[m:, n:]


def _strassen_left(a11, a12, a21, a22):
    return [a11 + a22, a21 + a22, a11, a22, a11 + a12, a21 - a11, a12 - a22]


def _strassen_right(b11, b12, b21, b22):
    return [b11 + b22, b11, b12 - b22, b21 - b11, b22, b11 + b12, b21 + b22]


def _strassen_combine(m):
    top = jnp.concatenate([m[0] + m[3] - m[4] + m[6], m[2] + m[4]], axis=1)
    bot = jnp.concatenate([m[1] + m[3], m[0] - m[1] + m[2] + m[5]], axis=1)
    return jnp.concatenate([top, bot], axis=0)


def _pack(x):
    return pltpu.bitcast(x, U32)


def _unpack(x):
    return pltpu.bitcast(x, BF16)


def _rows_max8(x):
    return jnp.max(x.reshape(x.shape[0] // 8, 8, x.shape[1]), axis=0)


def _abs_max8(x):
    a = jnp.abs(x)
    m = a[:, 0:128]
    for g in range(1, x.shape[1] // 128):
        m = jnp.maximum(m, a[:, g * 128:(g + 1) * 128])
    return _rows_max8(m)


def _lane_gather(x, idx):
    return jnp.take_along_axis(x, idx, axis=1, mode="promise_in_bounds")


def _lane_shift(x, n):
    lane = jax.lax.broadcasted_iota(jnp.int32, x.shape, 1)
    return _lane_gather(x, (lane + n) & 127)


def _lane_splat(x, n):
    return _lane_gather(x, jnp.full(x.shape, n, jnp.int32))


def _kernel(x_hbm, wqkv_hbm, wo_hbm, wg_hbm, wu_hbm, wd_hbm, o_hbm,
            x_s, wqkv_s, k_s, kp_s, qt_s, vt_s, kh0, kh1, kb0, kb1,
            kf_s, sc_s, pend_s, ot_s, l_s, r_s, on_s, ob_s,
            wo_s, wg_s, wu_s, wd_s, sg_s, su_s, sd_s, sp_s, sems, *, S, D, F):
    step = pl.program_id(0)
    G = D // 128
    NC = S // TK
    NT = S // TQ
    NG = TK // 8
    NJ = TQ // 128
    R = TQ // FSPLIT
    q_scale = (DH ** -0.5) * math.log2(math.e)
    nv = [NVP[c % len(NVP)] for c in range(NC)]
    starts = [sum(CHUNKS[:i]) for i in range(len(CHUNKS))]
    order = [(c, g) for c in range(NC) for g in reversed(range(nv[c], NG))]
    first = [sum(NG - nv[i] for i in range(c)) for c in range(NC + 1)]
    NS = len(order)
    assert NS % 2 == 0
    khs, tabs = (kh0, kh1), (kb0, kb1)

    x_parts = [(starts[i], CHUNKS[i]) for i in range(3)] + [(starts[3], S - starts[3])]
    x_copies = [
        pltpu.make_async_copy(x_hbm.at[pl.ds(r0, n)], x_s.at[pl.ds(r0, n)], sems.at[i])
        for i, (r0, n) in enumerate(x_parts)]
    wq_copy, wk_copy, wv_copy = [
        pltpu.make_async_copy(wqkv_hbm.at[:, pl.ds(i * D, D)], wqkv_s.at[i, pl.ds(0, D)],
                              sems.at[sem])
        for i, sem in enumerate((1, 4, 2))]
    ffn_copies = [
        pltpu.make_async_copy(src, dst.at[pl.ds(0, F)], sems.at[5])
        for src, dst in ((wg_hbm, wg_s), (wu_hbm, wu_s), (wd_hbm, wd_s))]
    wo_copy = pltpu.make_async_copy(wo_hbm, wo_s, sems.at[6])

    KD = (F // 256) * 256

    def weight_sums(src, dst, rows, operands, pace):
        m, n = rows // 2, D // 2
        z = jnp.minimum(step, 0)
        slabs = m // SLAB
        per = -(-slabs // len(pace))
        for i in range(slabs):
            g, r = divmod(i, per)
            r = (r * (pace[g].shape[0] // 16) // per) * 16
            src[pl.ds(src.shape[0] - 16, 16), 0:128] = pace[g][r:r + 16, 0:128].astype(BF16)
            rs = [pl.ds(pl.multiple_of(z + (r0 + i * SLAB), SLAB), SLAB) for r0 in (0, m)]
            quads = [src[r, pl.ds(c0, n)].astype(F32) for r in rs for c0 in (0, n)]
            sums = [t for t in operands(*quads) if not any(t is q for q in quads)]
            for j, t in enumerate(sums):
                dst[j, pl.ds(i * SLAB, SLAB), :] = t.astype(BF16)

    def weight_operands(src, dst, rows, plain):
        m, n = rows // 2, D // 2
        out, i = [], 0
        for j in range(7):
            if j in plain:
                r0, c0 = plain[j]
                out.append(src[pl.ds(r0 * m, m), pl.ds(c0 * n, n)])
            else:
                out.append(dst[i, pl.ds(0, m), :])
                i += 1
        return out

    def norm_rows(ci):
        xn = _layernorm(x_s[pl.ds(starts[ci], CHUNKS[ci]), :].astype(F32))
        if ci == 0:
            return xn.astype(BF16)
        return [a.astype(BF16) for a in _strassen_left(*_quads(xn))]

    def project(xn, i):
        if not isinstance(xn, list):
            y = _dot(xn, wqkv_s[i, 0:D, :])
            return y, [y[:, 128 * g:128 * (g + 1)] for g in range(G - 1)]
        ws = weight_operands(wqkv_s.at[i], sp_s.at[i], D, {1: (0, 0), 4: (1, 1)})
        ms = [None] * 7
        for j in QKV_ORDER:
            ms[j] = _dot(xn[j], ws[j])
        return _strassen_combine(ms), [ms[j] for j in QKV_ORDER]

    def proj_sums(i, pace):
        weight_sums(wqkv_s.at[i], sp_s.at[i], D, _strassen_right, pace)

    def project_k(ci, xn):
        r0, n = starts[ci], CHUNKS[ci]
        c0, c1 = r0 // TK, (r0 + n) // TK
        k, pace = project(xn, 1)
        kp = jnp.concatenate(
            [k[(c - c0) * TK + 8 * g:(c - c0) * TK + 8 * g + 8]
             for c, g in order[first[c0]:first[c1]]], axis=0)
        kp = _pack(kp.astype(BF16))
        prows = pl.ds(first[c0] * 4, (first[c1] - first[c0]) * 4)
        for g in range(G):
            k_s[g, pl.ds(r0, n), :] = k[:, g * 128:(g + 1) * 128]
            kp_s[g, prows, :] = kp[:, g * 128:(g + 1) * 128]
        kh0[prows, :] = kp[:, 0:128]
        for c in range(c0, c1):
            rows = k[(c - c0) * TK:(c - c0) * TK + 8 * nv[c], 0:128]
            for d in range(DH):
                kb0[c, d, 0:8 * nv[c], :] = _lane_splat(rows, d)
        return pace

    def project_q(ci, xn):
        q, pace = project(xn, 0)
        q = q * q_scale
        qt_s[:, :, pl.ds(starts[ci], CHUNKS[ci])] = q.T.reshape(H, DH, CHUNKS[ci])
        return pace

    def project_v(ci, xn):
        v, pace = project(xn, 2)
        vt_s[:, :, pl.ds(starts[ci], CHUNKS[ci])] = v.T.reshape(H, DH, CHUNKS[ci])
        return pace

    def store_sums(h, qi, cols):
        for j in range(NJ):
            l_s[qi * NJ + j, pl.ds(pl.multiple_of(h * 8, 8), 8), :] = cols[j]

    def vpu_scores(h, qi, c, j, kb, z):
        n = 8 * nv[c]
        cz = c + z
        cols = pl.ds(qi * TQ + j * 128, 128)
        acc = None
        for d in range(DH):
            t = kb[cz, d, 0:n, :] * qt_s[h, d:d + 1, cols]
            acc = t if acc is None else acc + t
        return acc

    def prep_piece(g, lane0, pc, kh, kb):
        if pc % 8 == 0:
            i, n = pc // 8, 4 * DH // 8
            lo, hi = (i * (NS // 2)) // n, ((i + 1) * (NS // 2)) // n
            rows = pl.ds(8 * lo, 8 * (hi - lo))
            kh[rows, :] = _lane_shift(kp_s[g, rows, :], lane0)
        d, part = divmod(pc, 4)
        cs = range(part * (NC // 4), (part + 1) * (NC // 4))
        col = _lane_splat(jnp.concatenate(
            [k_s[g, pl.ds(c * TK, 8 * nv[c]), :] for c in cs], axis=0), lane0 + d)
        r = 0
        for c in cs:
            kb[c, d, 0:8 * nv[c], :] = col[r:r + 8 * nv[c]]
            r += 8 * nv[c]

    def finish_pending(h, acc, top):
        n = 8 * nv[NC - 1]
        pt = jnp.concatenate([top, pend_s[pl.ds(n, TK - n), :]], axis=0)
        ot_s[NT - 1, h] = acc + _dot(vt_s[h, :, pl.ds((NC - 1) * TK, TK)], pt)

    def head_pair(jj, carry):
        lmin, lmax, acc_prev, top_prev = carry
        hs = (2 * jj, 2 * jj + 1)
        nxt = [jnp.minimum(h + 1, H - 1) for h in hs]
        nxt = [(h // HPG, (h % HPG) * DH) for h in nxt]
        zs = [jnp.minimum(jj, 0) * (j + 1) for j in range(NJ)]
        zero = zs[0].astype(F32)
        units = [(hh, qi) for hh in range(2) for qi in range(NT)]
        total = len(units) * NC
        slen = len(units) * NS
        ends = [(t // NC) * NS + first[t % NC + 1] for t in range(total)]
        cuts = [min(e + LEAD + (e + LEAD) % 2, slen) for e in ends]
        pieces = {}
        work = sum(nv) * NJ * len(units)
        done = 0
        for t in range(total):
            for j in range(NJ):
                pos = min((done * slen) // work + VOFF, cuts[t] - 1)
                if t == total - 1:
                    pos = slen - 1
                pieces.setdefault(pos, []).append((t, j))
                done += nv[t % NC]
        mxu_p = {}
        vpu_p = {}
        lacc = {}
        qhs = {}
        acc = None

        def add_sums(ui, js, p):
            if all((ui, j) in lacc for j in js):
                prev = [lacc[ui, j] for j in js]
                prev = prev[0] if len(js) == 1 else jnp.concatenate(prev, axis=1)
                p = jnp.concatenate([prev, p], axis=0)
                fresh = js
            else:
                fresh = [j for j in js if (ui, j) not in lacc]
            if p.shape[0] > 8:
                p = jnp.sum(p.reshape(p.shape[0] // 8, 8, p.shape[1]), axis=0)
            for i, j in enumerate(js):
                pj = p if len(js) == 1 else p[:, 128 * i:128 * (i + 1)]
                lacc[ui, j] = pj if j in fresh else lacc[ui, j] + pj

        def score_rows(lo, hi):
            ui = lo // NS
            hh, qi = units[ui]
            if ui not in qhs:
                qhs[ui] = qt_s[hs[hh], :, pl.ds(qi * TQ, TQ)].astype(BF16)
            kk = _unpack(khs[hh][pl.ds(4 * (lo - ui * NS), 4 * (hi - lo)), :])
            s = _dot(kk[:, 0:DH], qhs[ui])
            marks = sorted({lo, hi} | {i for i in pieces if lo < i < hi})
            for a, b in zip(marks[:-1], marks[1:]):
                for tv, j in pieces.get(a, ()):
                    hv, qv = units[tv // NC]
                    p = jnp.exp2(vpu_scores(hs[hv], qv, tv % NC, j, tabs[hv], zs[j]))
                    add_sums(tv // NC, [j], p)
                    vpu_p[tv, j] = p
                p = jnp.exp2(s[8 * (a - lo):8 * (b - lo)])
                add_sums(ui, list(range(NJ)), p)
                for i in range(a, b):
                    c, g = order[i - ui * NS]
                    mxu_p[ui * NC + c, g] = p[8 * (i - a):8 * (i - a + 1)]

        lo = 0
        for t in range(total + 1):
            if t < total:
                hi = cuts[t]
                cut = min(hi, (lo // NS + 1) * NS)
                if cut > lo:
                    score_rows(lo, cut)
                if hi > cut:
                    score_rows(cut, hi)
                lo = hi
                hh, qi = units[t // NC]
                for pc in range(4 * DH):
                    if FILL0 + (pc * (FILL1 - FILL0)) // (4 * DH) == qi * NC + t % NC:
                        prep_piece(*nxt[hh], pc, khs[1 - hh], tabs[1 - hh])
            if t == 0:
                finish_pending(jnp.maximum(hs[0] - 1, 0), acc_prev, top_prev)
                continue
            u = t - 1
            ui, c = divmod(u, NC)
            hh, qi = units[ui]
            h = hs[hh]
            top = jnp.concatenate([vpu_p.pop((u, j)) for j in range(NJ)], axis=1)
            rest = [mxu_p.pop((u, g)) for g in range(nv[c], NG)]
            if c == NC - 1:
                for j in range(NJ):
                    lmin = jnp.minimum(lmin, lacc[ui, j])
                    lmax = jnp.maximum(lmax, lacc[ui, j])
                store_sums(h, qi, [lacc[ui, j] for j in range(NJ)])
            if u == total - 1:
                pend_s[pl.ds(8 * nv[c], TK - 8 * nv[c]), :] = jnp.concatenate(rest, axis=0)
                return lmin, lmax, acc, top
            pt = jnp.concatenate([top] + rest, axis=0)
            acc = (zero if c == 0 else acc) + _dot(vt_s[h, :, pl.ds(c * TK, TK)], pt)
            if c == NC - 1:
                ot_s[qi, h] = acc

    def safe_head(h, carry):
        def shift_keys(c, carry):
            rows = pl.ds(pl.multiple_of(c * TK, TK), TK)
            kf_s[rows, :] = _lane_shift(k_s[h // HPG, rows, :], (h % HPG) * DH)
            return carry

        jax.lax.fori_loop(0, NC, shift_keys, 0)

        def tile(qi, carry):
            qh = qt_s[h, :, pl.ds(pl.multiple_of(qi * TQ, TQ), TQ)]

            def scores(c, m8):
                s = _dot(kf_s[pl.ds(pl.multiple_of(c * TS, TS), TS), :][:, 0:DH], qh)
                sc_s[c] = s
                return jnp.maximum(m8, _rows_max8(s))

            m8 = jax.lax.fori_loop(0, S // TS, scores, jnp.full((8, TQ), -jnp.inf, F32))
            m = jnp.max(m8, axis=0, keepdims=True)

            def weigh(c, st):
                acc, l8 = st
                p = jnp.exp2(sc_s[c] - m)
                v = vt_s[h, :, pl.ds(pl.multiple_of(c * TS, TS), TS)]
                return (acc + _dot(v, p),
                        l8 + jnp.sum(p.reshape(TS // 8, 8, TQ), axis=0))

            acc, l8 = jax.lax.fori_loop(
                0, S // TS, weigh, (jnp.zeros((DH, TQ), F32), jnp.zeros((8, TQ), F32)))
            ot_s[qi, h] = acc
            store_sums(h, qi, [l8[:, 128 * j:128 * (j + 1)] for j in range(NJ)])
            return carry

        return jax.lax.fori_loop(0, NT, tile, carry)

    def attn_rows(blk, b):
        js = range(b * R // 128, (b + 1) * R // 128)
        for j in js:
            l = l_s[blk * NJ + j, pl.ds(0, H, stride=8), :]
            for i in range(1, 8):
                l = l + l_s[blk * NJ + j, pl.ds(i, H, stride=8), :]
            r_s[:, 128 * j:128 * (j + 1)] = 1.0 / l
        heads = []
        for h in range(H):
            r = jnp.concatenate(
                [jnp.broadcast_to(r_s[h:h + 1, 128 * j:128 * (j + 1)], (8, 128))
                 for j in js], axis=1)
            heads.append(ot_s[blk, h, :, pl.ds(b * R, R)] * jnp.concatenate([r, r], axis=0))
        return jnp.concatenate(heads, axis=0).T.astype(BF16)

    def stage_attn(blk):
        on_s[...] = _pack(attn_rows(blk, 0))

    @pl.when(step == 0)
    def _():
        for cp in (x_copies[0], wk_copy, x_copies[1], wq_copy, wv_copy,
                   x_copies[2], x_copies[3], *ffn_copies, wo_copy):
            cp.start()
        pend_s[...] = jnp.zeros(pend_s.shape, F32)
        x_copies[0].wait()
        xn0 = norm_rows(0)
        wk_copy.wait()
        proj_sums(1, project_k(0, xn0))
        x_copies[1].wait()
        wq_copy.wait()
        proj_sums(0, project_q(0, xn0))
        xn1 = norm_rows(1)
        project_q(1, xn1)
        project_k(1, xn1)
        wv_copy.wait()
        x_copies[2].wait()
        proj_sums(2, project_v(0, xn0))
        project_v(1, xn1)
        wv8 = _abs_max8(wqkv_s[2, 0:D, :].astype(F32))
        xn2 = norm_rows(2)
        project_k(2, xn2)
        x_copies[3].wait()
        project_v(2, xn2)
        xn3 = norm_rows(3)
        project_v(3, xn3)
        project_q(2, xn2)
        xn4 = norm_rows(4)
        project_k(4, xn4)
        for cp in ffn_copies:
            cp.wait()
        weight_sums(wg_s, sg_s, F, _strassen_left, project_q(3, xn3))
        weight_sums(wu_s, su_s, F, _strassen_left, project_v(4, xn4))
        weight_sums(wd_s, sd_s, KD, _strassen_right, project_q(4, xn4))
        project_k(3, xn3)

        ones = jnp.ones((8, 128), F32)
        lmin, lmax, acc, top = jax.lax.fori_loop(
            0, H // 2, head_pair,
            (ones, ones, jnp.zeros((DH, TQ), F32), jnp.zeros((8 * nv[NC - 1], TQ), F32)))
        wo_copy.wait()
        finish_pending(H - 1, acc, top)
        stage_attn(0)
        worst = jnp.max(jnp.maximum(jnp.maximum(lmax, 1.0 / lmin) * (1.0 / SUM_LIMIT),
                                    wv8 * (D / VALUE_LIMIT)))

        @pl.when(jnp.logical_not(worst <= 1.0))
        def _():
            jax.lax.fori_loop(0, H, safe_head, 0)
            stage_attn(0)

    h1s, acts = [], []
    for b in range(FSPLIT):
        rows = pl.ds(pl.multiple_of(step * TQ + b * R, R), R)
        o = _unpack(on_s[...]) if b == 0 else attn_rows(step, b)
        h1s.append(x_s[rows, :].astype(F32) + _dot(o, wo_s[...]))
    stage_attn(jnp.minimum(step + 1, NT - 1))
    for b in range(FSPLIT):
        hn = _layernorm(h1s[b])
        if b == FSPLIT - 1:
            z = jnp.minimum(step, 0)
            tap = on_s[pl.ds(pl.multiple_of(z * 8, 8), 8), 0:128] & z.astype(U32)
            hp = pltpu.bitcast(hn, U32)
            top = jnp.concatenate([hp[0:8, 0:128] | tap, hp[0:8, 128:]], axis=1)
            hn = pltpu.bitcast(jnp.concatenate([top, hp[8:]], axis=0), F32)
        t11, t21, t12, t22 = _quads(hn)
        ts = [t.astype(BF16) for t in _strassen_right(t11, t12, t21, t22)]
        ws = [weight_operands(src, dst, F, {2: (0, 0), 3: (1, 1)})
              for src, dst in ((wg_s, sg_s), (wu_s, su_s))]
        ms = [[None] * 7, [None] * 7]
        for i in GU_ORDER:
            for k in range(2):
                ms[k][i] = _dot_nt(ws[k][i], ts[i])
        acts.append(_gelu_tanh(_strassen_combine(ms[0])) * _strassen_combine(ms[1]))

    def down(act_t):
        a11, a21, a12, a22 = _quads(act_t[0:KD])
        ls = [a.astype(BF16).T for a in _strassen_left(a11, a12, a21, a22)]
        ws = weight_operands(wd_s, sd_s, KD, {1: (0, 0), 4: (1, 1)})
        tail = _dot(act_t[KD:].astype(BF16).T, wd_s[KD:F, :])
        ms = [None] * 7
        for i in DOWN_ORDER:
            ms[i] = _dot(ls[i], ws[i])
        return tail + _strassen_combine(ms)

    def out_copy(r0):
        rows = pl.ds(r0, R // 2)
        return pltpu.make_async_copy(ob_s.at[rows], o_hbm.at[rows], sems.at[7])

    for b in range(FSPLIT):
        y = (h1s[b] + down(acts[b])).astype(ob_s.dtype)
        for i in range(2):
            r0 = pl.multiple_of(step * TQ + b * R + i * (R // 2), R // 2)
            ob_s[pl.ds(r0, R // 2), :] = y[i * (R // 2):(i + 1) * (R // 2)]
            out_copy(r0).start()

    @pl.when(step == NT - 1)
    def _():
        for i in range(2 * S // R):
            out_copy(i * (R // 2)).wait()


@jax.jit
def pallas_sequential_preLN__softmax_full_mha__geglu_ffn__prompt_kernel(
    A_x: jax.Array,
    A_wqkv: jax.Array,
    A_wo: jax.Array,
    B_x: jax.Array,
    B_w_gate: jax.Array,
    B_w_up: jax.Array,
    B_w_down: jax.Array,
):
    B, S, D = A_x.shape
    F = B_w_gate.shape[1]
    assert B == 1 and D == H * DH and sum(CHUNKS) == S
    G = D // 128
    NC = S // TK
    NT = S // TQ
    FP = -(-(F // 2) // 32) * 32
    hbm = pl.BlockSpec(memory_space=pltpu.MemorySpace.HBM)

    out = pl.pallas_call(
        functools.partial(_kernel, S=S, D=D, F=F),
        grid=(NT,),
        in_specs=[hbm] * 6,
        out_specs=hbm,
        out_shape=jax.ShapeDtypeStruct((S, D), A_x.dtype),
        scratch_shapes=[
            pltpu.VMEM((S, D), BF16),
            pltpu.VMEM((3, D + 16, D), BF16),
            pltpu.VMEM((G, S, 128), F32),
            pltpu.VMEM((G, S // 2, 128), U32),
            pltpu.VMEM((H, DH, S), F32),
            pltpu.VMEM((H, DH, S), F32),
            pltpu.VMEM((S // 2, 128), U32),
            pltpu.VMEM((S // 2, 128), U32),
            pltpu.VMEM((NC, DH, 8 * max(NVP), 128), F32),
            pltpu.VMEM((NC, DH, 8 * max(NVP), 128), F32),
            pltpu.VMEM((S, 128), F32),
            pltpu.VMEM((S // TS, TS, TQ), F32),
            pltpu.VMEM((TK, TQ), F32),
            pltpu.VMEM((NT, H, DH, TQ), F32),
            pltpu.VMEM((S // 128, H * 8, 128), F32),
            pltpu.VMEM((H, TQ), F32),
            pltpu.VMEM((TQ // FSPLIT // 2, D), U32),
            pltpu.VMEM((S, D), A_x.dtype),
            pltpu.VMEM((D, D), BF16),
            pltpu.VMEM((F + 16, D), BF16),
            pltpu.VMEM((F + 16, D), BF16),
            pltpu.VMEM((F + 16, D), BF16),
            pltpu.VMEM((5, FP, D // 2), BF16),
            pltpu.VMEM((5, FP, D // 2), BF16),
            pltpu.VMEM((5, (F // 256) * 128, D // 2), BF16),
            pltpu.VMEM((3, 5, D // 2, D // 2), BF16),
            pltpu.SemaphoreType.DMA((8,)),
        ],
        compiler_params=pltpu.CompilerParams(
            dimension_semantics=("arbitrary",),
            vmem_limit_bytes=100 * 1024 * 1024,
        ),
    )(A_x.reshape(S, D), A_wqkv, A_wo, B_w_gate.T, B_w_up.T, B_w_down)
    return out.reshape(B, S, D)
```
